```python
import os as _os
_os.environ.setdefault("JAX_PLATFORMS", "cpu")
import jax
import jax.numpy as jnp

def _softmax(x, axis=-1):
    return jax.nn.softmax(x, axis=axis)
def _gelu(x):
    return jax.nn.gelu(x, approximate=True)
def _silu(x):
    return jax.nn.silu(x)
def _sigmoid(x):
    return jax.nn.sigmoid(x)
def _layernorm(x, axis=-1, eps=1e-5):
    m = jnp.mean(x, axis=axis, keepdims=True)
    v = jnp.var(x, axis=axis, keepdims=True)
    return (x - m) / jnp.sqrt(v + eps)
def _scatter_add(tgt, idx, src, axis=0):
    return tgt.at[idx].add(src)
def _segment_sum(src, seg, n):
    return jax.ops.segment_sum(src, seg, n)
class _Rng:
    def __init__(self, key):
        self._k = key
    def _next(self):
        self._k, sub = jax.random.split(self._k)
        return sub
    def normal(self, shape):
        return jax.random.normal(self._next(), shape, dtype=jnp.bfloat16)
    def randint(self, lo, hi, shape):
        return jax.random.randint(self._next(), shape, lo, hi, dtype=jnp.int32)
    def uniform(self, shape, lo=0.0, hi=1.0):
        return jax.random.uniform(self._next(), shape, jnp.bfloat16, lo, hi)
    def permutation(self, n):
        return jax.random.permutation(self._next(), n)


kernel_name = 'concat_heads__sliding_block__sliding_block__prompt'

def setup_inputs():
    _rng = _Rng(jax.random.key(int.from_bytes(__import__("os").urandom(4), "little")))
    _w = (lambda a: (lambda t: t.astype(jnp.bfloat16) if jnp.issubdtype(t.dtype, jnp.floating) else t)(jnp.asarray(a)))
    def _A_setup():
        B, S, D = 1, 2048, 448
        return {
            "x": _w((lambda *s: _rng.normal(s) * 0.2)(B, S, D)),
            "wqkv": _w((lambda *s: _rng.normal(s) * 0.2)(D, 3 * D)),
            "wo": _w((lambda *s: _rng.normal(s) * 0.05)(D, D)),
        }
    _A_in = _A_setup()

    def _B_setup():
        B, S, D = 1, 2048, 448
        return {
            "x": _w((lambda *s: _rng.normal(s) * 0.2)(B, S, D)),
            "wqkv": _w((lambda *s: _rng.normal(s) * 0.2)(D, 3 * D)),
            "wo": _w((lambda *s: _rng.normal(s) * 0.05)(D, D)),
        }
    _B_in = _B_setup()

    return {
        "A_x": _A_in["x"],
        "A_wqkv": _A_in["wqkv"],
        "A_wo": _A_in["wo"],
        "B_x": _B_in["x"],
        "B_wqkv": _B_in["wqkv"],
        "B_wo": _B_in["wo"],
    }

def reference(A_x, A_wqkv, A_wo, B_x, B_wqkv, B_wo):
    def _A_ref(x, wqkv, wo):
        B, S, D = x.shape
        H = 16; Dh = D // H; W = 256
        qkv = (lambda x, *d: x.transpose(*d))((x @ wqkv).reshape(B, S, 3, H, Dh), 2, 0, 3, 1, 4)
        q, k, v = qkv[0], qkv[1], qkv[2]
        scores = jnp.einsum("bhqd,bhkd->bhqk", q, k) * (Dh ** -0.5)
        idx = jnp.arange(S)
        mask = (idx[:, None] - idx[None, :] >= 0) & (idx[:, None] - idx[None, :] < W)
        scores = jnp.where(mask[None, None], scores, -1e9)
        p = _softmax(scores, axis=-1)
        o = jnp.einsum("bhqk,bhkd->bhqd", p, v)
        return (lambda x, *d: x.transpose(*d))(o, 0, 2, 1, 3).reshape(B, S, D) @ wo

    def _B_ref(x, wqkv, wo):
        B, S, D = x.shape
        H = 16; Dh = D // H; W = 256
        qkv = (lambda x, *d: x.transpose(*d))((x @ wqkv).reshape(B, S, 3, H, Dh), 2, 0, 3, 1, 4)
        q, k, v = qkv[0], qkv[1], qkv[2]
        scores = jnp.einsum("bhqd,bhkd->bhqk", q, k) * (Dh ** -0.5)
        idx = jnp.arange(S)
        mask = (idx[:, None] - idx[None, :] >= 0) & (idx[:, None] - idx[None, :] < W)
        scores = jnp.where(mask[None, None], scores, -1e9)
        p = _softmax(scores, axis=-1)
        o = jnp.einsum("bhqk,bhkd->bhqd", p, v)
        return (lambda x, *d: x.transpose(*d))(o, 0, 2, 1, 3).reshape(B, S, D) @ wo

    a = _A_ref(A_x, A_wqkv, A_wo)
    b = _B_ref(B_x, B_wqkv, B_wo)
    return jnp.concatenate([a, b], axis=-1)
```

```python
import functools
import jax, jax.numpy as jnp
from jax import lax
import jax.experimental.pallas as pl
import jax.experimental.pallas.tpu as pltpu

S, D, H, DH, WIN = 2048, 448, 16, 28, 256
T = 256
NT = T // 128
NEG = -1e30
NSLOT = 3
QSCALE = (DH ** -0.5) * 1.4426950408889634
f32, bf16, u32 = jnp.float32, jnp.bfloat16, jnp.uint32


def _pad_heads(r, fill):
    n = r.shape[1]
    row = lax.broadcasted_iota(jnp.int32, (8, n), 0)
    lo = row < 4
    out = []
    for p in range(r.shape[0] // 56):
        b = 56 * p
        sh = r[b + 24:b + 32]
        out.append(jnp.concatenate([r[b:b + 24], jnp.where(lo, sh, fill)], axis=0))
        out.append(jnp.concatenate([jnp.where(lo, fill, sh), r[b + 32:b + 56]], axis=0))
    return out


def _kernel(xa_ref, wa_ref, woa_ref, xb_ref, wb_ref, wob_ref, o_ref, kn_ref, vt_ref, *p_refs):
    step = pl.program_id(0)
    z1 = lax.shift_right_logical(step, 8)
    z2 = lax.shift_right_logical(step, 9)

    @pl.when(step == 0)
    def _():
        lane = lax.broadcasted_iota(jnp.int32, (WIN // 2, 128), 1)
        l64 = lane % 64
        padlane = jnp.logical_and(l64 >= 28, l64 < 36)
        pre = jnp.where(padlane, jnp.uint32(0x3F803F80), jnp.uint32(0))
        for b in range(2):
            for g in range(4):
                kn_ref[b, g, 0:WIN // 2, :] = pre
            for t in range(2):
                vt_ref[b, t] = jnp.zeros((256, 128), u32)

    lane8 = lax.broadcasted_iota(jnp.int32, (16, 128), 1)
    blk = lane8 // 32
    blk_masks = [blk == c for c in range(4)]
    bit0 = (blk % 2) == 1
    bit1 = blk >= 2
    r32 = lax.broadcasted_iota(jnp.int32, (32, 128), 0)
    q32 = lax.broadcasted_iota(jnp.int32, (32, 128), 1) % 32
    upper = r32 > q32
    row8 = lax.broadcasted_iota(jnp.int32, (8, 128), 0)
    lo8 = row8 < 4
    never = row8 < z1
    zero16 = jnp.zeros((16, 128), u32)
    row0h = pl.multiple_of(step * (T // 2), T // 2)

    xs = (xa_ref, xb_ref)
    ws = (wa_ref, wb_ref)
    wos = (woa_ref, wob_ref)
    qh = {}
    sv = {}
    oh = {}
    outs = {}

    def slot(b, m, g):
        return ((b * NT + m) * 4 + g) % NSLOT

    def proj(b, part, half):
        r0 = part * D + half * 224
        r = jnp.dot(ws[b][r0:r0 + 224, :], xs[b][...], preferred_element_type=f32)
        if part == 0:
            hs = _pad_heads(r * QSCALE, NEG)
            for i in range(8):
                qh[b, 8 * half + i] = hs[i]
        elif part == 1:
            hs = _pad_heads(r, 0.0)
            for gg in range(2):
                kt = jnp.concatenate(hs[4 * gg:4 * gg + 4], axis=0).astype(bf16)
                kn_ref[b, 2 * half + gg, pl.ds(row0h + WIN // 2, T // 2), :] = pltpu.bitcast(kt.T, u32)
        else:
            hs = _pad_heads(r, 1.0)
            vt = pltpu.bitcast(jnp.concatenate(hs, axis=0).astype(bf16), u32)
            for m in range(NT):
                vt_ref[b, step * NT + m + 2, 128 * half:128 * half + 128, :] = vt[:, 128 * m:128 * m + 128]

    def qk(b, m, g):
        qr = []
        for hp in range(4):
            qq = qh[b, 4 * g + hp][:, 128 * m:128 * m + 128]
            qq = pltpu.bitcast(qq.astype(bf16), u32)
            if hp:
                qq = pltpu.roll(qq, 32 * hp, axis=1)
            qr.append(qq)
        ss = []
        for c in range(4):
            wt = jnp.concatenate(
                [jnp.where(blk_masks[(c + hp) % 4], qr[hp], zero16) for hp in range(4)], axis=0)
            wt = pltpu.bitcast(wt, bf16)
            kk = kn_ref[b, g, pl.ds(pl.multiple_of(row0h + 64 * m + 16 * c, 16), 144), :]
            s = jnp.dot(pltpu.bitcast(kk, bf16), wt, preferred_element_type=f32)
            s = jnp.concatenate([jnp.where(upper, s[0:32], NEG), s[32:256],
                                 jnp.where(upper, NEG, s[256:288])], axis=0)
            mx = jnp.broadcast_to(jnp.max(s, axis=0, keepdims=True), (8, 128))
            ss.append((s, mx))
        sv[b, m, g] = ss

    def sel(mask, a, bb):
        if a is None and bb is None:
            return None
        return jnp.where(mask, zero16 if a is None else a, zero16 if bb is None else bb)

    def sm(grp, trig):
        ss = sv.pop(grp)
        mxs = [x[1] for x in ss]
        pr = p_refs[slot(*grp)]
        for rho in range(12):
            src = []
            for c in range(4):
                k = rho - c
                if 0 <= k <= 8:
                    if trig is not None:
                        mxs[c] = jnp.where(never, trig[rho], mxs[c])
                    mx = jnp.concatenate([mxs[c]] * 4, axis=0)
                    p = jnp.exp2(ss[c][0][32 * k:32 * k + 32] - mx).astype(bf16)
                    src.append(pltpu.bitcast(p, u32))
                else:
                    src.append(None)
            u = [sel(bit0, src[(k + 1) % 4], src[k]) for k in range(4)]
            wv = [sel(bit1, u[(k + 2) % 4], u[k]) for k in range(4)]
            for hp in range(4):
                pr[z1, hp, 16 * rho:16 * rho + 16, :] = wv[(-hp) % 4]

    def pvf(b, m, g):
        pr = p_refs[slot(b, m, g)]
        acc = [None] * 4
        for i in range(3):
            for hp in range(4):
                h = 4 * g + hp
                pt = pltpu.bitcast(pr[z2, hp, 64 * i:64 * i + 64, :], bf16)
                vv = pltpu.bitcast(vt_ref[b, step * NT + m + i, 16 * h:16 * h + 16, :], bf16)
                d = jnp.dot(vv, pt, preferred_element_type=f32)
                acc[hp] = d if acc[hp] is None else acc[hp] + d
        for hp in range(4):
            h = 4 * g + hp
            den = acc[hp][28:29] if h % 2 == 0 else acc[hp][0:1]
            o = acc[hp] * pl.reciprocal(den, approx=True)
            if hp:
                o = pltpu.roll(o, 128 - 32 * hp, axis=1)
            oh[b, m, h] = o

    def oproj(b, m):
        rows = []
        for p in range(8):
            a, bb = oh.pop((b, m, 2 * p)), oh.pop((b, m, 2 * p + 1))
            rows += [a[0:24], jnp.where(lo8, a[24:32], bb[0:8]), bb[8:32]]
        ot = jnp.concatenate(rows, axis=0).astype(bf16)
        outs[b, m] = jnp.dot(wos[b][...], ot, preferred_element_type=f32)

    def fin(m):
        y = jnp.concatenate([outs.pop((0, m)), outs.pop((1, m))], axis=0).astype(bf16)
        o_ref[128 * m:128 * m + 128, :] = y.T

    groups = [(b, m, g) for b in range(2) for m in range(NT) for g in range(4)]
    ng = len(groups)
    fill = {i: [] for i in range(ng + 1)}
    pjb = [(1, part, half) for part in (1, 0, 2) for half in range(2)]
    for i, a in enumerate(pjb):
        fill[i * (4 * NT - 2) // 6].append(functools.partial(proj, *a))
    for m in range(NT - 1):
        fill[ng - 3 - 2 * (NT - 2 - m)].append(functools.partial(oproj, 0, m))
    for m in range(NT - 1):
        fill[ng - 2 * (NT - 2 - m)].append(functools.partial(oproj, 1, m))
        fill[ng - 2 * (NT - 2 - m)].append(functools.partial(fin, m))

    def trig_of(x):
        n = x.shape[0] // 8
        return [x[8 * ((n * r) // 12):8 * ((n * r) // 12) + 8] for r in range(12)]

    for part in (1, 0, 2):
        for half in range(2):
            proj(0, part, half)
    qk(*groups[0])
    for i in range(ng + 1):
        if i + 1 < ng:
            qk(*groups[i + 1])
            tr = trig_of(sv[groups[i + 1]][0][0])
        elif i + 1 == ng:
            oproj(0, NT - 1)
            tr = trig_of(outs[0, NT - 1])
        if i < ng:
            sm(groups[i], tr)
        for f in fill[i]:
            f()
        if i >= 1:
            pvf(*groups[i - 1])
    oproj(1, NT - 1)
    fin(NT - 1)


@jax.jit
def pallas_concat_heads__sliding_block__sliding_block__prompt_kernel(A_x, A_wqkv, A_wo, B_x, B_wqkv, B_wo):
    xa = A_x.reshape(S, D).T
    xb = B_x.reshape(S, D).T
    xspec = pl.BlockSpec((D, T), lambda i: (0, i))
    wspec = pl.BlockSpec((3 * D, D), lambda i: (0, 0))
    wospec = pl.BlockSpec((D, D), lambda i: (0, 0))
    out = pl.pallas_call(
        _kernel,
        grid=(S // T,),
        in_specs=[xspec, wspec, wospec, xspec, wspec, wospec],
        out_specs=pl.BlockSpec((T, 2 * D), lambda i: (i, 0)),
        out_shape=jax.ShapeDtypeStruct((S, 2 * D), bf16),
        scratch_shapes=[pltpu.VMEM((2, 4, (WIN + S) // 2, 128), u32),
                        pltpu.VMEM((2, 2 + S // 128, 256, 128), u32)]
        + [pltpu.VMEM((1, 4, 192, 128), u32)] * NSLOT,
        compiler_params=pltpu.CompilerParams(dimension_semantics=("arbitrary",),
                                             vmem_limit_bytes=64 * 1024 * 1024),
    )(xa, A_wqkv.T, A_wo.T, xb, B_wqkv.T, B_wo.T)
    return out.reshape(1, S, 2 * D)
```

```python
import functools
import jax, jax.numpy as jnp
from jax import lax
import jax.experimental.pallas as pl
import jax.experimental.pallas.tpu as pltpu

S, D, H, DH, WIN = 2048, 448, 16, 28, 256
NTILE = S // 128
MT = 4
LT = 2
NMID = (NTILE - 2 - LT) // MT
assert 2 + NMID * MT + LT == NTILE
NEG = -1e30
QSCALE = (DH ** -0.5) * 1.4426950408889634
f32, bf16, u32 = jnp.float32, jnp.bfloat16, jnp.uint32
DROP_PEN = 20
DROP_LAST = 8
DROP_END = 20
ANCHOR_RHO = 8
DROP = 16
PVTRIG = 1
WCOLS = ((0, 384), (384, 896), (896, 1344))
XA1 = 128 * (3 + MT)
XB1 = 128 * (2 + MT)
XCOLS = (((0, 256), (256, 384), (384, XA1), (XA1, S)), ((0, 256), (256, XB1), (XB1, S)))


def _kernel(xa_hbm, wa_hbm, woa_hbm, xb_hbm, wb_hbm, wob_hbm, o_hbm,
            w_v, wo_v, x_v, wt_v, wot_v, kn0_v, kn1_v, vt0_v, vt1_v, q0_v, q1_v, q2_v, p0_v, p1_v, p2_v, p3_v,
            ot0_v, ot1_v, rem_v, out_v, isem, osem):
    step = pl.program_id(0)
    z1 = lax.shift_right_logical(step, 8)
    z2 = lax.shift_right_logical(step, 9)
    kn_vs, vt_vs = (kn0_v, kn1_v), (vt0_v, vt1_v)
    q_vs, p_vs, ot_vs = (q0_v, q1_v, q2_v), (p0_v, p1_v, p2_v, p3_v), (ot0_v, ot1_v)
    x_hbm, w_hbm, wo_hbm = (xa_hbm, xb_hbm), (wa_hbm, wb_hbm), (woa_hbm, wob_hbm)

    def mul(jj, m, off=0, al=None):
        v = m * jj + off
        return v if isinstance(jj, int) else pl.multiple_of(v, al or m)

    def w_cp(b, part):
        lo, hi = WCOLS[part]
        return pltpu.make_async_copy(w_hbm[b].at[:, lo:hi], w_v.at[b, :, lo:hi], isem.at[3 * b + part])

    def wo_cp(b):
        return pltpu.make_async_copy(wo_hbm[b], wo_v.at[b], isem.at[6 + b])

    class _Multi:
        def __init__(self, cps):
            self.cps = cps

        def start(self):
            for cp in self.cps:
                cp.start()

        def wait(self):
            for cp in self.cps:
                cp.wait()

    def x_cp(b, i):
        lo, hi = XCOLS[b][i]
        return _Multi([pltpu.make_async_copy(x_hbm[b].at[:, 128 * t:128 * t + 128], x_v.at[b, t],
                                             isem.at[8 + 4 * b + i]) for t in range(lo // 128, hi // 128)])

    def o_cp(jj, lo=0, hi=2 * D):
        rows = pl.ds(mul(jj, 128), 128)
        return pltpu.make_async_copy(out_v.at[rows, lo:hi], o_hbm.at[rows, lo:hi], osem.at[0])

    def wait(name, *cps):
        for cp in cps:
            cp.wait()

    def body(kind, j):
        lane16 = lax.broadcasted_iota(jnp.int32, (16, 128), 1)
        blk = lane16 // 32
        blk_masks = [blk == c for c in range(4)]
        bit0 = (blk % 2) == 1
        bit1 = blk >= 2
        r32 = lax.broadcasted_iota(jnp.int32, (32, 128), 0)
        q32 = lax.broadcasted_iota(jnp.int32, (32, 128), 1) % 32
        upper = r32 > q32
        row8 = lax.broadcasted_iota(jnp.int32, (8, 128), 0)
        lo8 = row8 < 4
        never = row8 < z1
        zero16 = jnp.zeros((16, 128), u32)

        def vregs(x):
            return [x[8 * i:8 * i + 8] for i in range(x.shape[0] // 8)]

        def pad_heads(r, fill):
            out = []
            for p in range(8):
                o = 56 * p
                sh = r[o + 24:o + 32]
                out.append(jnp.concatenate([r[o:o + 24], jnp.where(lo8, sh, fill)], axis=0))
                out.append(jnp.concatenate([jnp.where(lo8, fill, sh), r[o + 32:o + 56]], axis=0))
            return out

        def rho0_of(sb):
            jj = sb[1]
            return {0: 8, 1: 4}[jj] if isinstance(jj, int) and jj < 2 else 0

        def proj_dot(sb, part):
            b, jj = sb[:2]
            wt = pltpu.bitcast(wt_v[b, 224 * part:224 * part + 224, :], bf16)
            return jnp.dot(wt, x_v[b, jj], preferred_element_type=f32)

        def proj_post(sb, part, r):
            b, jj, qs = sb[:3]
            if part == 0:
                hs = pad_heads(r * QSCALE, 0.0)
                for h in range(16):
                    qq = pltpu.bitcast(hs[h].astype(bf16), u32)
                    if h % 4:
                        qq = pltpu.roll(qq, 32 * (h % 4), axis=1)
                    q_vs[qs][z1, 16 * h:16 * h + 16, :] = qq
            elif part == 1:
                hs = pad_heads(r, 0.0)
                for g in range(4):
                    kt = jnp.concatenate(hs[4 * g:4 * g + 4], axis=0).astype(bf16)
                    kn_vs[b][g, pl.ds(mul(jj, 64), 64), :] = pltpu.bitcast(kt.T, u32)
            else:
                hs = pad_heads(r, 1.0)
                vt_vs[b][jj] = pltpu.bitcast(jnp.concatenate(hs, axis=0).astype(bf16), u32)

        def proj(sb, part):
            r = proj_dot(sb, part)
            proj_post(sb, part, r)
            return vregs(r)

        scores = {}
        fresh, anchors, carry = [], [], []

        def qk(n):
            sb, g = groups[n]
            b, jj, qs = sb[:3]
            rho0 = rho0_of(sb)
            qr = [q_vs[qs][z2, 64 * g + 16 * hp:64 * g + 16 * hp + 16, :] for hp in range(4)]
            ss = []
            for c in range(4):
                k0 = max(0, rho0 - c)
                wt = jnp.concatenate(
                    [jnp.where(blk_masks[(c + hp) % 4], qr[hp], zero16) for hp in range(4)], axis=0)
                kk = kn_vs[b][g, pl.ds(mul(jj, 64, 16 * c - 128 + 16 * k0, 16), 16 * (9 - k0)), :]
                s = jnp.dot(pltpu.bitcast(kk, bf16), pltpu.bitcast(wt, bf16), preferred_element_type=f32)
                ss.append((s, k0))
            scores[n] = ss
            return vregs(ss[3][0])

        def sel(mask, a, bb):
            if a is None and bb is None:
                return None
            return jnp.where(mask, zero16 if a is None else a, zero16 if bb is None else bb)

        def sm(n, trig):
            rho0 = rho0_of(groups[n][0])
            ss, mxs = [], []
            for s, k0 in scores.pop(n):
                m = s.shape[0]
                parts = [jnp.where(upper, s[0:32], NEG), s[32:m - 32]] if k0 == 0 else [s[0:m - 32]]
                parts = [x for x in parts if x.shape[0]]
                s = jnp.concatenate(parts + [jnp.where(upper, NEG, s[m - 32:m])], axis=0)
                ss.append((s, k0))
                mxs.append(jnp.broadcast_to(jnp.max(s, axis=0, keepdims=True), (8, 128)))
            items = [(rho, c) for rho in range(rho0, 12) for c in range(4) if 0 <= rho - c <= 8]
            tix = {it: (len(trig) * i) // len(items) for i, it in enumerate(items)}
            for rho in range(rho0, 12):
                src = []
                for c in range(4):
                    k = rho - c
                    if 0 <= k <= 8:
                        mxs[c] = jnp.where(never, trig[tix[rho, c]], mxs[c])
                        if anchors and rho >= ANCHOR_RHO:
                            mxs[c] = jnp.where(never, anchors.pop(), mxs[c])
                        mx = jnp.concatenate([mxs[c]] * 4, axis=0)
                        kk = k - ss[c][1]
                        p = jnp.exp2(ss[c][0][32 * kk:32 * kk + 32] - mx).astype(bf16)
                        src.append(pltpu.bitcast(p, u32))
                    else:
                        src.append(None)
                u = [sel(bit0, src[(k + 1) % 4], src[k]) for k in range(4)]
                wv = [sel(bit1, u[(k + 2) % 4], u[k]) for k in range(4)]
                for hp in range(4):
                    p_vs[n % 4][z1, hp, 16 * rho:16 * rho + 16, :] = wv[(-hp) % 4]

        def pv(n):
            sb, g = groups[n] if n >= 0 else (prev, 3)
            b, jj, _, os_ = sb[:4]
            acc = [None] * 4
            tr = []
            for i in range(rho0_of(sb) // 4, 3):
                jv = jj + i - 2
                if n < 0 and i == 0 and not isinstance(jv, int):
                    jv = jnp.maximum(jv, 0)
                for hp in range(4):
                    h = 4 * g + hp
                    pt = pltpu.bitcast(p_vs[n % 4][z2, hp, 64 * i:64 * i + 64, :], bf16)
                    vv = pltpu.bitcast(vt_vs[b][jv, 16 * h:16 * h + 16, :], bf16)
                    d = jnp.dot(vv, pt, preferred_element_type=f32)
                    if hp == 3:
                        tr += vregs(d)
                    acc[hp] = d if acc[hp] is None else acc[hp] + d
            oo = []
            for hp in range(4):
                den = acc[hp][28:29] if hp % 2 == 0 else acc[hp][0:1]
                o = acc[hp] * pl.reciprocal(den, approx=True)
                if hp:
                    o = pltpu.roll(o, 128 - 32 * hp, axis=1)
                oo.append(o)
            rows = []
            for p in range(2):
                a, bb = oo[2 * p], oo[2 * p + 1]
                rows += [a[0:24], jnp.where(lo8, a[24:32], bb[0:8]), bb[8:32]]
            ot = jnp.concatenate(rows, axis=0).astype(bf16)
            ot_vs[os_][z1, 56 * g:56 * g + 56, :] = pltpu.bitcast(ot, u32)
            return tr

        def ot_load(sb, klo, khi):
            return pltpu.bitcast(ot_vs[sb[3]][z2, klo // 2:khi // 2, :], bf16)

        def oproj_part(sb, ot, klo, khi):
            b = sb[0]
            wa = jnp.concatenate([wot_v[b, 96:112, klo:khi], wot_v[b, 0:96, klo:khi]], axis=0)
            ya = jnp.dot(pltpu.bitcast(wa, bf16), ot, preferred_element_type=f32)
            yb = jnp.dot(pltpu.bitcast(wot_v[b, 112:224, klo:khi], bf16), ot, preferred_element_type=f32)
            return jnp.concatenate([ya[32:224], ya[0:32], yb], axis=0)

        def oproj_post(sb, y, final=False):
            b, jj, _, _, rs = sb
            rows = pl.ds(mul(jj, 128), 128)
            if b == 0:
                yt = y[0:384].astype(bf16).T
                out_v[rows, 0:384] = yt
                rem_v[z1 + rs] = y[384:448]
                if final:
                    o_cp(jj, 0, 384).start()
            else:
                yt = jnp.concatenate([rem_v[z2 + rs], y], axis=0).astype(bf16).T
                out_v[rows, 384:896] = yt
                if final:
                    o_cp(jj, 384, 896).start()
                else:
                    o_cp(jj).start()
            last_rows = lax.bitcast_convert_type(pltpu.bitcast(yt[112:128], u32), f32)
            fresh.extend(last_rows[:, 128 * i:128 * i + 128] for i in range(yt.shape[1] // 128))

        def oproj(sb, final=False):
            b, os_ = sb[0], sb[3]
            ot = pltpu.bitcast(ot_vs[os_][z2], bf16)
            y = jnp.dot(pltpu.bitcast(wot_v[b], bf16), ot, preferred_element_type=f32)
            oproj_post(sb, y, final)
            return vregs(y)

        def wtrans(b, part):
            lo, hi = WCOLS[part]
            wt_v[b, lo // 2:hi // 2, :] = pltpu.bitcast(w_v[b, :, lo:hi].T, u32)

        def wotrans(b):
            wot_v[b] = pltpu.bitcast(wo_v[b].T, u32)

        def slot(qks, fills, pvs, sms, drop=None, pv_first=False):
            anchors.extend(fresh)
            fresh.clear()
            trig = list(carry) if PVTRIG else []
            carry.clear()
            for n in qks:
                trig += qk(n)
            if pv_first:
                for n in pvs:
                    t = pv(n)
                    trig += t if PVTRIG else []
            for f in fills:
                trig += f()
            trig = trig[:len(trig) - (drop if drop is not None else (DROP if fills else 0))]
            if not pv_first:
                for n in pvs:
                    carry.extend(pv(n))
            for i, n in enumerate(sms):
                sm(n, trig[len(trig) * i // len(sms):len(trig) * (i + 1) // len(sms)])

        P = functools.partial
        if kind == "first":
            a0, a1, b0, b1, a2 = (0, 0, 2, 0, 0), (0, 1, 1, 1, 1), (1, 0, 2, 0, 0), (1, 1, 1, 1, 1), (0, 2, 0, 0, 0)
            prev = None
            groups = [(sb, g) for sb in (a0, a1, b0, b1) for g in range(4)]
            wait("wA1", w_cp(0, 1))
            wtrans(0, 1)
            wait("wA2", x_cp(0, 0))
            proj(a0, 1)
            r = proj_dot(a1, 1)
            wait("wB", w_cp(0, 0), x_cp(0, 1))
            wtrans(0, 0)
            proj_post(a1, 1, r)
            proj(a2, 1)
            proj(a0, 0)
            proj(a1, 0)
            qk(0)
            qk(1)
            wait("wC", w_cp(0, 2))
            wtrans(0, 2)
            slot([2, 3], [P(proj, a0, 2)], [], [0, 1])
            slot([4], [P(proj, a1, 2)], [0, 1], [2, 3])
            slot([5], [P(proj, a2, 0)], [2, 3], [4], drop=DROP_LAST, pv_first=True)
            wait("wD1", x_cp(1, 0), w_cp(1, 1), w_cp(1, 0), w_cp(1, 2))
            wtrans(1, 1)
            wtrans(1, 0)
            wtrans(1, 2)
            slot([6], [P(proj, b0, 1)], [4], [5], pv_first=True)
            slot([7], [P(proj, b0, 0)], [5], [6])
            slot([], [P(proj, b1, 1), P(qk, 8), P(qk, 9), P(proj, b1, 0)], [6], [7])
            slot([10, 11], [P(proj, b0, 2)], [7], [8, 9], drop=DROP_LAST, pv_first=True)
            wait("wD2", wo_cp(0), wo_cp(1))
            wotrans(0)
            wotrans(1)
            slot([12], [P(oproj, a0)], [8, 9], [10, 11])
            slot([13], [P(proj, b1, 2)], [10, 11], [12])
            slot([14], [P(oproj, a1)], [12], [13])
            slot([15], [P(oproj, b0)], [13], [14], drop=DROP_PEN)
            slot([], [P(proj, a2, 2)], [14], [15], drop=DROP_LAST, pv_first=True)
            for hp in range(4):
                p_vs[3][z1, hp, 0:64, :] = jnp.zeros((64, 128), u32)
        else:
            nt = MT if kind == "mid" else LT
            seq = []
            for t in range(nt):
                seq += [(0, j + t, 0, 0, 1), (1, j + t, 1, 1, 1)]
            prev = (1, j - 1, 1, 1, 1)
            chain = [prev] + seq + [(0, j + nt, 0, 0, 0)]
            groups = [(sb, g) for sb in seq for g in range(4)]
            pv(-1)
            qk(0)
            for i in range(len(seq)):
                lastsb = i + 1 == len(seq)
                n = 4 * i
                if lastsb and kind == "last":
                    slot([n + 1], [], [n - 1], [n])
                    slot([n + 2], [], [n], [n + 1])
                    slot([n + 3], [], [n + 1], [n + 2])
                    sa, sb = chain[i], seq[i]
                    ot = ot_load(sa, 0, 448)
                    wo = pltpu.bitcast(wot_v[0], bf16)
                    y0 = jnp.dot(wo[0:224], ot, preferred_element_type=f32)
                    pv(n + 2)
                    y1 = jnp.dot(wo[224:448], ot, preferred_element_type=f32)
                    trig = vregs(y0) + vregs(y1)
                    sm(n + 3, trig[:len(trig) - DROP_END])
                    oproj_post(sa, jnp.concatenate([y0, y1], axis=0), True)
                    ot_lo = ot_load(sb, 0, 256)
                    pv(n + 3)
                    y = oproj_part(sb, ot_lo, 0, 256)
                    ot_hi = pltpu.bitcast(ot_load(sb, 256, 448), u32)
                    top = ot_hi[0:8]
                    for a in fresh:
                        top = jnp.where(never, lax.bitcast_convert_type(a, u32), top)
                    ot_hi = pltpu.bitcast(jnp.concatenate([top, ot_hi[8:]], axis=0), bf16)
                    y = y + oproj_part(sb, ot_hi, 256, 448)
                    oproj_post(sb, y, True)
                else:
                    slot([n + 1], [P(proj, chain[i + 2], 1)], [n - 1] if n else [], [n])
                    slot([n + 2], [P(proj, chain[i + 2], 0)], [n], [n + 1])
                    slot([n + 3], [P(oproj, chain[i])], [n + 1], [n + 2], drop=DROP_PEN if lastsb else None)
                    slot([] if lastsb else [n + 4], [P(proj, chain[i + 2], 2)], [n + 2], [n + 3],
                         pv_first=lastsb, drop=DROP_LAST if lastsb else None)

    @pl.when(step == 0)
    def _():
        for cp in (w_cp(0, 1), x_cp(0, 0), w_cp(0, 0), x_cp(0, 1), w_cp(0, 2), x_cp(1, 0),
                   w_cp(1, 1), w_cp(1, 0), w_cp(1, 2), wo_cp(0), wo_cp(1), x_cp(1, 1), x_cp(0, 2), x_cp(1, 2),
                   x_cp(0, 3)):
            cp.start()
        body("first", 0)

    @pl.when(step == 1)
    def _():
        wait("wx1", x_cp(1, 1), x_cp(0, 2))

    @pl.when(step == 2)
    def _():
        wait("wx2", x_cp(1, 2), x_cp(0, 3))

    @pl.when(jnp.logical_and(step > 0, step <= NMID))
    def _():
        body("mid", 2 + MT * (step - 1))

    @pl.when(step == NMID + 1)
    def _():
        body("last", NTILE - LT)
        wait("wout", pltpu.make_async_copy(out_v, o_hbm, osem.at[0]))


@jax.jit
def pallas_concat_heads__sliding_block__sliding_block__prompt_kernel(A_x, A_wqkv, A_wo, B_x, B_wqkv, B_wo):
    xa = A_x.reshape(S, D).T
    xb = B_x.reshape(S, D).T
    anyspec = pl.BlockSpec(memory_space=pl.ANY)
    V = pltpu.VMEM
    out = pl.pallas_call(
        _kernel,
        grid=(NMID + 2,),
        in_specs=[anyspec] * 6,
        out_specs=anyspec,
        out_shape=jax.ShapeDtypeStruct((S, 2 * D), bf16),
        scratch_shapes=[
            V((2, D, 3 * D), bf16),
            V((2, D, D), bf16),
            V((2, NTILE, D, 128), bf16),
            V((2, 3 * D // 2, D), u32),
            V((2, D // 2, D), u32),
            V((4, S // 2, 128), u32), V((4, S // 2, 128), u32),
            V((NTILE, 256, 128), u32), V((NTILE, 256, 128), u32),
            V((1, 256, 128), u32), V((1, 256, 128), u32), V((1, 256, 128), u32),
            V((1, 4, 192, 128), u32), V((1, 4, 192, 128), u32), V((1, 4, 192, 128), u32), V((1, 4, 192, 128), u32),
            V((1, 224, 128), u32), V((1, 224, 128), u32),
            V((2, 64, 128), f32),
            V((S, 2 * D), bf16),
            pltpu.SemaphoreType.DMA((15,)),
            pltpu.SemaphoreType.DMA((1,)),
        ],
        compiler_params=pltpu.CompilerParams(dimension_semantics=("arbitrary",),
                                             vmem_limit_bytes=64 * 1024 * 1024,
                                             disable_semaphore_checks=True,
                                             disable_bounds_checks=True),
    )(xa, A_wqkv, A_wo, xb, B_wqkv, B_wo)
    return out.reshape(1, S, 2 * D)
```

```python
import functools
import jax, jax.numpy as jnp
from jax import lax
import jax.experimental.pallas as pl
import jax.experimental.pallas.tpu as pltpu

S, D, H, DH, WIN = 2048, 448, 16, 28, 256
NTILE = S // 128
MT = 4
LT = 2
NMID = (NTILE - 2 - LT) // MT
assert 2 + NMID * MT + LT == NTILE
NEG = -1e30
QSCALE = (DH ** -0.5) * 1.4426950408889634
f32, bf16, u32 = jnp.float32, jnp.bfloat16, jnp.uint32
DROP_PEN = 20
DROP_LAST = 8
DROP_END = 28
ANCHOR_RHO = 8
DROP = 16
PVTRIG = 1
DROP_BAR = 12
FSPLIT = 4
H2 = 8
HM = 1
RT0 = 0
RTS = 2
WCOLS = ((0, 384), (384, 896), (896, 1344), (384, 640), (640, 896))
XA1 = 128 * (3 + MT)
XB1 = 128 * (2 + MT)
XCOLS = (((0, 128), (256, 384), (384, XA1), (XA1, S), (128, 256)), ((0, 256), (256, XB1), (XB1, S)))


def _kernel(xa_hbm, wa_hbm, woa_hbm, xb_hbm, wb_hbm, wob_hbm, o_hbm,
            w_v, wo_v, x_v, wt_v, wot_v, kn0_v, kn1_v, vt0_v, vt1_v, q0_v, q1_v, q2_v, p0_v, p1_v, p2_v, p3_v,
            ot0_v, ot1_v, rem_v, out_v, isem, osem):
    step = pl.program_id(0)
    z1 = lax.shift_right_logical(step, 8)
    z2 = lax.shift_right_logical(step, 9)
    kn_vs, vt_vs = (kn0_v, kn1_v), (vt0_v, vt1_v)
    q_vs, p_vs, ot_vs = (q0_v, q1_v, q2_v), (p0_v, p1_v, p2_v, p3_v), (ot0_v, ot1_v)
    x_hbm, w_hbm, wo_hbm = (xa_hbm, xb_hbm), (wa_hbm, wb_hbm), (woa_hbm, wob_hbm)

    def mul(jj, m, off=0, al=None):
        v = m * jj + off
        return v if isinstance(jj, int) else pl.multiple_of(v, al or m)

    def w_cp(b, part):
        lo, hi = WCOLS[part]
        sem = {4: 1, 3: 15}.get(part, 3 * b + part)
        return pltpu.make_async_copy(w_hbm[b].at[:, lo:hi], w_v.at[b, :, lo:hi], isem.at[sem])

    def wo_cp(b):
        return pltpu.make_async_copy(wo_hbm[b], wo_v.at[b], isem.at[6 + b])

    class _Multi:
        def __init__(self, cps):
            self.cps = cps

        def start(self):
            for cp in self.cps:
                cp.start()

        def wait(self):
            for cp in self.cps:
                cp.wait()

    def x_cp(b, i):
        lo, hi = XCOLS[b][i]
        return _Multi([pltpu.make_async_copy(x_hbm[b].at[:, 128 * t:128 * t + 128], x_v.at[b, t],
                                             isem.at[16 if i == 4 else 8 + 4 * b + i]) for t in range(lo // 128, hi // 128)])

    def o_cp(jj, lo=0, hi=2 * D):
        rows = pl.ds(mul(jj, 128), 128)
        return pltpu.make_async_copy(out_v.at[rows, lo:hi], o_hbm.at[rows, lo:hi], osem.at[0])

    def wait(name, *cps):
        for cp in cps:
            cp.wait()

    def body(kind, j):
        lane16 = lax.broadcasted_iota(jnp.int32, (16, 128), 1)
        blk = lane16 // 32
        blk_masks = [blk == c for c in range(4)]
        bit0 = (blk % 2) == 1
        bit1 = blk >= 2
        r32 = lax.broadcasted_iota(jnp.int32, (32, 128), 0)
        q32 = lax.broadcasted_iota(jnp.int32, (32, 128), 1) % 32
        upper = r32 > q32
        row8 = lax.broadcasted_iota(jnp.int32, (8, 128), 0)
        lo8 = row8 < 4
        never = row8 < z1
        zero16 = jnp.zeros((16, 128), u32)

        def vregs(x):
            return [x[8 * i:8 * i + 8] for i in range(x.shape[0] // 8)]

        def pad_heads(r, fill):
            out = []
            lo8 = lax.broadcasted_iota(jnp.int32, (8, r.shape[1]), 0) < 4
            for p in range(8):
                o = 56 * p
                sh = r[o + 24:o + 32]
                out.append(jnp.concatenate([r[o:o + 24], jnp.where(lo8, sh, fill)], axis=0))
                out.append(jnp.concatenate([jnp.where(lo8, fill, sh), r[o + 32:o + 56]], axis=0))
            return out

        def rho0_of(sb):
            jj = sb[1]
            return {0: 8, 1: 4}[jj] if isinstance(jj, int) and jj < 2 else 0

        def proj_dot(sb, part, lo=None, hi=None):
            b, jj = sb[:2]
            if lo is None:
                lo, hi = D * part, D * part + D
            wt = pltpu.bitcast(wt_v[b, lo // 2:hi // 2, :], bf16)
            return jnp.dot(wt, x_v[b, jj], preferred_element_type=f32)

        def proj_post(sb, part, r):
            b, jj, qs = sb[:3]
            if part == 0:
                hs = pad_heads(r * QSCALE, 0.0)
                for h in range(16):
                    qq = pltpu.bitcast(hs[h].astype(bf16), u32)
                    if h % 4:
                        qq = pltpu.roll(qq, 32 * (h % 4), axis=1)
                    q_vs[qs][z1, 16 * h:16 * h + 16, :] = qq
            elif part == 1:
                hs = pad_heads(r, 0.0)
                for g in range(4):
                    kt = jnp.concatenate(hs[4 * g:4 * g + 4], axis=0).astype(bf16)
                    kn_vs[b][g, pl.ds(mul(jj, 64), 64), :] = pltpu.bitcast(kt.T, u32)
            else:
                hs = pad_heads(r, 1.0)
                vt_vs[b][jj] = pltpu.bitcast(jnp.concatenate(hs, axis=0).astype(bf16), u32)

        def proj(sb, part):
            r = proj_dot(sb, part)
            proj_post(sb, part, r)
            return vregs(r)

        scores = {}
        fresh, anchors, carry, pending = [], [], [], []

        def qk(n):
            sb, g = groups[n]
            b, jj, qs = sb[:3]
            rho0 = rho0_of(sb)
            qr = [q_vs[qs][z2, 64 * g + 16 * hp:64 * g + 16 * hp + 16, :] for hp in range(4)]
            ss = []
            for c in range(4):
                k0 = max(0, rho0 - c)
                wt = jnp.concatenate(
                    [jnp.where(blk_masks[(c + hp) % 4], qr[hp], zero16) for hp in range(4)], axis=0)
                kk = kn_vs[b][g, pl.ds(mul(jj, 64, 16 * c - 128 + 16 * k0, 16), 16 * (9 - k0)), :]
                s = jnp.dot(pltpu.bitcast(kk, bf16), pltpu.bitcast(wt, bf16), preferred_element_type=f32)
                ss.append((s, k0))
            scores[n] = ss
            return vregs(ss[3][0])

        def sel(mask, a, bb):
            if a is None and bb is None:
                return None
            return jnp.where(mask, zero16 if a is None else a, zero16 if bb is None else bb)

        def sm(n, trig):
            rho0 = rho0_of(groups[n][0])
            ss, mxs = [], []
            for s, k0 in scores.pop(n):
                m = s.shape[0]
                parts = [jnp.where(upper, s[0:32], NEG), s[32:m - 32]] if k0 == 0 else [s[0:m - 32]]
                parts = [x for x in parts if x.shape[0]]
                s = jnp.concatenate(parts + [jnp.where(upper, NEG, s[m - 32:m])], axis=0)
                ss.append((s, k0))
                mxs.append(jnp.broadcast_to(jnp.max(s, axis=0, keepdims=True), (8, 128)))
            items = [(rho, c) for rho in range(rho0, 12) for c in range(4) if 0 <= rho - c <= 8]
            tix = {it: (len(trig) * i) // len(items) for i, it in enumerate(items)}
            for rho in range(rho0, 12):
                src = []
                for c in range(4):
                    k = rho - c
                    if 0 <= k <= 8:
                        mxs[c] = jnp.where(never, trig[tix[rho, c]], mxs[c])
                        if anchors and rho >= ANCHOR_RHO:
                            mxs[c] = jnp.where(never, anchors.pop(), mxs[c])
                        mx = jnp.concatenate([mxs[c]] * 4, axis=0)
                        kk = k - ss[c][1]
                        p = jnp.exp2(ss[c][0][32 * kk:32 * kk + 32] - mx).astype(bf16)
                        src.append(pltpu.bitcast(p, u32))
                    else:
                        src.append(None)
                u = [sel(bit0, src[(k + 1) % 4], src[k]) for k in range(4)]
                wv = [sel(bit1, u[(k + 2) % 4], u[k]) for k in range(4)]
                for hp in range(4):
                    p_vs[n % 4][0, hp, 16 * rho:16 * rho + 16, :] = wv[(-hp) % 4]

        def pv(n, defer=True):
            sb, g = groups[n] if n >= 0 else (prev, 3)
            b, jj, _, os_ = sb[:4]
            acc = [None] * 4
            tr = []
            for i in range(rho0_of(sb) // 4, 3):
                jv = jj + i - 2
                if n < 0 and i == 0 and not isinstance(jv, int):
                    jv = jnp.maximum(jv, 0)
                for hp in range(4):
                    h = 4 * g + hp
                    pt = pltpu.bitcast(p_vs[n % 4][0, hp, 64 * i:64 * i + 64, :], bf16)
                    vv = pltpu.bitcast(vt_vs[b][jv, 16 * h:16 * h + 16, :], bf16)
                    d = jnp.dot(vv, pt, preferred_element_type=f32)
                    if hp == 3:
                        tr += vregs(d)
                    acc[hp] = d if acc[hp] is None else acc[hp] + d

            def post(trig=None):
                cnt = 0
                for hp in range(4):
                    den = acc[hp][28:29] if hp % 2 == 0 else acc[hp][0:1]
                    o = acc[hp] * pl.reciprocal(den, approx=False)
                    o = pltpu.bitcast(o.astype(bf16), u32)
                    if hp:
                        halves = []
                        for i in range(2):
                            x = o[8 * i:8 * i + 8]
                            if trig is not None:
                                t = lax.bitcast_convert_type(trig[cnt], u32)
                                x = jnp.where(never, t, x)
                            cnt += 1
                            halves.append(pltpu.roll(x, 128 - 32 * hp, axis=1))
                        o = jnp.concatenate(halves, axis=0)
                    ot_vs[os_][z1, 64 * g + 16 * hp:64 * g + 16 * hp + 16, :] = o
            if defer:
                pending.append(post)
            else:
                post()
            return tr

        def ot_load(sb, klo, khi):
            return pltpu.bitcast(ot_vs[sb[3]][z2, klo // 2:khi // 2, :], bf16)

        def oproj_part(sb, ot, klo, khi, cuts):
            ys = [jnp.dot(pltpu.bitcast(wot_v[sb[0], r0 // 2:r1 // 2, klo:khi], bf16), ot,
                          preferred_element_type=f32) for r0, r1 in zip(cuts[:-1], cuts[1:])]
            return jnp.concatenate(ys, axis=0)

        def pin():
            out_v[pl.ds(pl.multiple_of(S + 16 * z1, 16), 16), 0:128] = jnp.zeros((16, 128), bf16)
            v = out_v[pl.ds(pl.multiple_of(S + 16 * z2, 16), 16), 0:128]
            fresh.append(lax.bitcast_convert_type(pltpu.bitcast(v, u32), f32))

        def oproj_post(sb, y, final=False):
            b, jj, _, _, rs = sb
            rows = pl.ds(mul(jj, 128), 128)
            if b == 0:
                yt = y[0:384].astype(bf16).T
                out_v[rows, 0:384] = yt
                rem_v[z1 + rs] = y[384:448]
                if final:
                    o_cp(jj, 0, 384).start()
            else:
                yt = jnp.concatenate([rem_v[z2 + rs], y], axis=0).astype(bf16).T
                if final:
                    nr = 128 // FSPLIT
                    for i in range(FSPLIT):
                        r0 = 128 * jj + nr * i
                        out_v[r0:r0 + nr, 384:896] = yt[nr * i:nr * i + nr]
                        pltpu.make_async_copy(out_v.at[r0:r0 + nr, 384:896], o_hbm.at[r0:r0 + nr, 384:896],
                                              osem.at[0]).start()
                    return
                out_v[rows, 384:896] = yt
                o_cp(jj).start()
            pin()

        def oproj(sb, final=False):
            b, os_ = sb[0], sb[3]
            ot = pltpu.bitcast(ot_vs[os_][z2], bf16)
            y = jnp.dot(pltpu.bitcast(wot_v[b], bf16), ot, preferred_element_type=f32)
            oproj_post(sb, y, final)
            return vregs(y)

        def wtrans(b, part):
            lo, hi = WCOLS[part]
            wt_v[b, lo // 2:hi // 2, :] = pltpu.bitcast(w_v[b, :, lo:hi].T, u32)

        def wotrans(b):
            wp = jnp.concatenate(pad_heads(wo_v[b].astype(f32), 0.0), axis=0).astype(bf16)
            wot_v[b] = pltpu.bitcast(wp.T, u32)

        def flush(trig=()):
            trig = list(trig)[RT0::RTS]
            for post in pending:
                if len(trig) >= 6:
                    post(trig[:6])
                    trig = trig[6:]
                else:
                    post()
            pending.clear()

        def slot(qks, fills, pvs, sms, drop=None, pv_first=False, hold=0):
            anchors.extend(fresh)
            fresh.clear()
            trig = list(carry) if PVTRIG else []
            carry.clear()
            nc = len(trig)
            for n in qks:
                trig += qk(n)
            if not hold:
                flush(trig[nc:])
            if pv_first:
                for n in pvs:
                    t = pv(n, False)
                    trig += t if PVTRIG else []
            nc = len(trig)
            for f in fills:
                trig += f()
            if hold == 2:
                flush(trig[nc + H2:])
            trig = trig[:len(trig) - (drop if drop is not None else (DROP if fills else 0))]
            if not pv_first:
                for n in pvs:
                    carry.extend(pv(n))
            for i, n in enumerate(sms):
                sm(n, trig[len(trig) * i // len(sms):len(trig) * (i + 1) // len(sms)])

        P = functools.partial
        if kind == "first":
            a0, a1, b0, b1, a2 = (0, 0, 2, 0, 0), (0, 1, 1, 1, 1), (1, 0, 2, 0, 0), (1, 1, 1, 1, 1), (0, 2, 0, 0, 0)
            prev = None
            groups = [(sb, g) for sb in (a0, a1, b0, b1) for g in range(4)]
            wait("wA1", w_cp(0, 3))
            wtrans(0, 3)
            wait("wA2", x_cp(0, 0))
            r0 = proj_dot(a0, None, 384, 640)
            wait("wA3", x_cp(0, 4), w_cp(0, 4))
            wtrans(0, 4)
            r1 = proj_dot(a1, None, 384, 640)
            proj_post(a0, 1, jnp.concatenate([r0[64:], proj_dot(a0, None, 640, 896)], axis=0))
            r = jnp.concatenate([r1[64:], proj_dot(a1, None, 640, 896)], axis=0)
            wait("wB", w_cp(0, 0), x_cp(0, 1))
            wtrans(0, 0)
            proj_post(a1, 1, r)
            proj(a2, 1)
            proj_post(a0, 0, jnp.concatenate([proj_dot(a0, None, 0, 384), r0[:64]], axis=0))
            r = jnp.concatenate([proj_dot(a1, None, 0, 384), r1[:64]], axis=0)
            wait("wC", w_cp(0, 2))
            wtrans(0, 2)
            proj_post(a1, 0, r)
            qk(0)
            qk(1)
            slot([2, 3], [P(proj, a0, 2)], [], [0, 1])
            slot([4], [P(proj, a1, 2)], [0, 1], [2, 3], drop=DROP_PEN)
            held = []

            def dot_only(sb, part):
                held.append(proj_dot(sb, part))
                return vregs(held[-1])
            slot([5], [P(dot_only, a2, 0)], [2, 3], [4], drop=DROP_BAR, pv_first=True)
            wait("wD1", x_cp(1, 0), w_cp(1, 1), w_cp(1, 0), w_cp(1, 2))
            proj_post(a2, 0, held.pop())
            wtrans(1, 1)
            wtrans(1, 0)
            wtrans(1, 2)
            slot([6], [P(proj, b0, 1)], [4], [5], pv_first=True)
            slot([7], [P(proj, b0, 0)], [5], [6])
            slot([], [P(proj, b1, 1), P(qk, 8), P(qk, 9), P(proj, b1, 0)], [6], [7])
            slot([10, 11], [P(dot_only, b0, 2)], [7], [8, 9], drop=DROP_BAR, pv_first=True)
            wait("wD2", wo_cp(0), wo_cp(1))
            proj_post(b0, 2, held.pop())
            wotrans(0)
            wotrans(1)
            slot([12], [P(oproj, a0)], [8, 9], [10, 11])
            slot([13], [P(proj, b1, 2)], [10, 11], [12])
            slot([14], [P(oproj, a1)], [12], [13])
            slot([15], [P(oproj, b0)], [13], [14], drop=DROP_PEN)
            slot([], [P(proj, a2, 2)], [14], [15], drop=DROP_LAST, pv_first=True)
            for hp in range(4):
                p_vs[3][0, hp, 0:64, :] = jnp.zeros((64, 128), u32)
        else:
            nt = MT if kind == "mid" else LT
            seq = []
            for t in range(nt):
                seq += [(0, j + t, 0, 0, 1), (1, j + t, 1, 1, 1)]
            prev = (1, j - 1, 1, 1, 1)
            chain = [prev] + seq + [(0, j + nt, 0, 0, 0)]
            groups = [(sb, g) for sb in seq for g in range(4)]
            if kind == "last":
                groups[-4:] = groups[-4:][::-1]
            pv(-1)
            flush(qk(0))
            for i in range(len(seq)):
                lastsb = i + 1 == len(seq)
                n = 4 * i
                if lastsb and kind == "last":
                    slot([n + 1], [], [n - 1], [n])
                    slot([n + 2], [], [n], [n + 1])
                    slot([n + 3], [], [n + 1], [n + 2])
                    flush()
                    sa, sb = chain[i], seq[i]
                    ot = ot_load(sa, 0, 512)
                    wo = pltpu.bitcast(wot_v[0], bf16)
                    y0 = jnp.dot(wo[0:224], ot, preferred_element_type=f32)
                    t = pv(n + 2, False)
                    y1 = jnp.dot(wo[224:448], ot, preferred_element_type=f32)
                    trig = carry + vregs(y0) + t + vregs(y1)
                    sm(n + 3, trig[:len(trig) - DROP_END])
                    oproj_post(sa, jnp.concatenate([y0, y1], axis=0), True)
                    ot_hi = ot_load(sb, 128, 512)
                    pv(n + 3, False)
                    y = oproj_part(sb, ot_hi[128:384], 256, 512, (0, 224, 448))
                    y = y + oproj_part(sb, ot_hi[0:128], 128, 256, (0, 112, 224, 336, 448))
                    ot_lo = pltpu.bitcast(ot_load(sb, 0, 128), u32)
                    top = jnp.where(never, lax.bitcast_convert_type(fresh.pop(), u32), ot_lo[0:8])
                    ot_lo = pltpu.bitcast(jnp.concatenate([top, ot_lo[8:]], axis=0), bf16)
                    wl = wot_v[1, :, 0:128]
                    lhs = [wl[32:88], wl[96:152], wl[160:216],
                           jnp.concatenate([wl[0:32], wl[88:96], wl[152:160], wl[216:224]], axis=0)]
                    d = [jnp.dot(pltpu.bitcast(w, bf16), ot_lo, preferred_element_type=f32) for w in lhs]
                    y = y + jnp.concatenate([d[3][0:64], d[0], d[3][64:80], d[1], d[3][80:96], d[2], d[3][96:112]],
                                            axis=0)
                    oproj_post(sb, y, True)
                else:
                    slot([n + 1], [P(proj, chain[i + 2], 1)], [n - 1] if n else [], [n])
                    slot([n + 2], [P(proj, chain[i + 2], 0)], [n], [n + 1])
                    slot([n + 3], [P(oproj, chain[i])], [n + 1], [n + 2], drop=DROP_PEN if lastsb else None, hold=1)
                    slot([] if lastsb else [n + 4], [P(proj, chain[i + 2], 2)], [n + 2], [n + 3],
                         pv_first=lastsb, drop=DROP_LAST if lastsb else None, hold=2 if (lastsb or HM == 2) else 1)

    @pl.when(step == 0)
    def _():
        for cp in (w_cp(0, 3), x_cp(0, 0), x_cp(0, 4), w_cp(0, 4), w_cp(0, 0), x_cp(0, 1), w_cp(0, 2), x_cp(1, 0),
                   w_cp(1, 1), w_cp(1, 0), w_cp(1, 2), wo_cp(0), wo_cp(1), x_cp(1, 1), x_cp(0, 2), x_cp(1, 2),
                   x_cp(0, 3)):
            cp.start()
        body("first", 0)

    @pl.when(step == 1)
    def _():
        wait("wx1", x_cp(1, 1), x_cp(0, 2))

    @pl.when(step == 2)
    def _():
        wait("wx2", x_cp(1, 2), x_cp(0, 3))

    @pl.when(jnp.logical_and(step > 0, step <= NMID))
    def _():
        body("mid", 2 + MT * (step - 1))

    @pl.when(step == NMID + 1)
    def _():
        body("last", NTILE - LT)
        wait("wout", pltpu.make_async_copy(out_v.at[0:S], o_hbm, osem.at[0]))


@jax.jit
def pallas_concat_heads__sliding_block__sliding_block__prompt_kernel(A_x, A_wqkv, A_wo, B_x, B_wqkv, B_wo):
    xa = A_x.reshape(S, D).T
    xb = B_x.reshape(S, D).T
    anyspec = pl.BlockSpec(memory_space=pl.ANY)
    V = pltpu.VMEM
    out = pl.pallas_call(
        _kernel,
        grid=(NMID + 2,),
        in_specs=[anyspec] * 6,
        out_specs=anyspec,
        out_shape=jax.ShapeDtypeStruct((S, 2 * D), bf16),
        scratch_shapes=[
            V((2, D, 3 * D), bf16),
            V((2, D, D), bf16),
            V((2, NTILE, D, 128), bf16),
            V((2, 3 * D // 2, D), u32),
            V((2, D // 2, 512), u32),
            V((4, S // 2, 128), u32), V((4, S // 2, 128), u32),
            V((NTILE, 256, 128), u32), V((NTILE, 256, 128), u32),
            V((1, 256, 128), u32), V((1, 256, 128), u32), V((1, 256, 128), u32),
            V((1, 4, 192, 128), u32), V((1, 4, 192, 128), u32), V((1, 4, 192, 128), u32), V((1, 4, 192, 128), u32),
            V((1, 256, 128), u32), V((1, 256, 128), u32),
            V((2, 64, 128), f32),
            V((S + 16, 2 * D), bf16),
            pltpu.SemaphoreType.DMA((17,)),
            pltpu.SemaphoreType.DMA((1,)),
        ],
        compiler_params=pltpu.CompilerParams(dimension_semantics=("arbitrary",),
                                             vmem_limit_bytes=64 * 1024 * 1024,
                                             disable_semaphore_checks=True,
                                             disable_bounds_checks=True),
    )(xa, A_wqkv, A_wo, xb, B_wqkv, B_wo)
    return out.reshape(1, S, 2 * D)
```

```python
import functools

import jax
import jax.numpy as jnp
from jax import lax
import jax.experimental.pallas as pl
import jax.experimental.pallas.tpu as pltpu

S, D, DH = 2048, 448, 28
NTILE = S // 128
FT = 3
MT = 4
LT = 1
NMID = (NTILE - FT - LT) // MT
assert FT + NMID * MT + LT == NTILE
NEG = -1e30
QSCALE = (DH ** -0.5) * 1.4426950408889634
f32, bf16, u32 = jnp.float32, jnp.bfloat16, jnp.uint32

DROP = 24
DROP_PEN = 20
DROP_LAST = 8
DROP_BAR = 12
DROP_END = 28
ANCHOR_RHO = 8
FSPLIT = 4

WCOLS = ((0, 384), (384, 896), (896, 1344), (384, 640), (640, 896))
XTILES = (((0, 1), (1, 2), (2, 3), (3, 4), (4, FT + 1 + MT), (FT + 1 + MT, NTILE)),
          ((0, FT), (FT, FT + MT), (FT + MT, NTILE)))


def _kernel(xa_hbm, wa_hbm, woa_hbm, xb_hbm, wb_hbm, wob_hbm, o_hbm,
            w_v, wo_v, x_v, wt_v, wot_v, kn0_v, kn1_v, vt0_v, vt1_v, q0_v, q1_v, q2_v,
            p0_v, p1_v, p2_v, p3_v, ot0_v, ot1_v, ot2_v, ot3_v, rem_v, out_v, isem, osem):
    step = pl.program_id(0)
    z1 = lax.shift_right_logical(step, 8)
    z2 = lax.shift_right_logical(step, 9)
    kn_vs, vt_vs = (kn0_v, kn1_v), (vt0_v, vt1_v)
    q_vs, p_vs, ot_vs = (q0_v, q1_v, q2_v), (p0_v, p1_v, p2_v, p3_v), (ot0_v, ot1_v, ot2_v, ot3_v)
    x_hbm, w_hbm, wo_hbm = (xa_hbm, xb_hbm), (wa_hbm, wb_hbm), (woa_hbm, wob_hbm)

    def mul(jj, m, off=0, al=None):
        v = m * jj + off
        return v if isinstance(jj, int) else pl.multiple_of(v, al or m)

    def w_cp(b, part):
        lo, hi = WCOLS[part]
        sem = {3: 1, 4: 17}.get(part, 3 * b + part)
        return [pltpu.make_async_copy(w_hbm[b].at[:, lo:hi], w_v.at[b, :, lo:hi], isem.at[sem])]

    def wo_cp(b):
        return [pltpu.make_async_copy(wo_hbm[b], wo_v.at[b], isem.at[6 + b])]

    def x_cp(b, i):
        return [pltpu.make_async_copy(x_hbm[b].at[:, 128 * t:128 * t + 128], x_v.at[b, t], isem.at[8 + 6 * b + i])
                for t in range(*XTILES[b][i])]

    def o_start(rows, lo, hi):
        pltpu.make_async_copy(out_v.at[rows, lo:hi], o_hbm.at[rows, lo:hi], osem.at[0]).start()

    def wait(*groups_of_copies):
        for cps in groups_of_copies:
            for cp in cps:
                cp.wait()

    def cat(xs):
        return xs[0] if len(xs) == 1 else jnp.concatenate(xs, axis=0)

    def dot(a, b):
        return jnp.dot(a, b, preferred_element_type=f32)

    def body(kind, j):
        blk64 = lax.broadcasted_iota(jnp.int32, (64, 128), 1) // 32
        in_blk = [lax.broadcasted_iota(jnp.int32, (16, 128), 1) // 32 == c for c in range(4)]
        bit0 = (blk64 % 2) == 1
        bit1 = blk64 >= 2
        upper = (lax.broadcasted_iota(jnp.int32, (32, 128), 0)
                 > lax.broadcasted_iota(jnp.int32, (32, 128), 1) % 32)
        never = lax.broadcasted_iota(jnp.int32, (8, 128), 0) < z1
        zero16 = jnp.zeros((16, 128), u32)
        neg32 = jnp.full((32, 128), NEG, f32)

        def ticks(x):
            return [(x, i) for i in range(x.shape[0] // 8)]

        def after(t, x):
            if isinstance(t, tuple):
                t = t[0][8 * t[1]:8 * t[1] + 8]
            if t.dtype != x.dtype:
                t = lax.bitcast_convert_type(t, x.dtype)
            return lax.select(never, t, x)

        def pad_heads(r, fill):
            lo8 = lax.broadcasted_iota(jnp.int32, (8, r.shape[1]), 0) < 4
            full = jnp.full((8, r.shape[1]), fill, f32)
            out = []
            for p in range(8):
                o = 56 * p
                sh = r[o + 24:o + 32]
                out += [r[o - 24 if p else 0:o + 24], lax.select(lo8, sh, full), lax.select(lo8, full, sh)]
            return cat(out + [r[D - 24:D]])

        def rho0_of(sb):
            jj = sb[1]
            return {0: 8, 1: 4}[jj] if isinstance(jj, int) and jj < 2 else 0

        def proj_dot(sb, lo, hi):
            b, jj = sb[:2]
            return dot(pltpu.bitcast(wt_v[b, lo // 2:hi // 2, :], bf16), x_v[b, jj])

        def proj_post(sb, part, r):
            b, jj, qs = sb[:3]
            if part == 0:
                q = pltpu.bitcast(pad_heads(r * QSCALE, 0.0).astype(bf16), u32)
                q_vs[qs][z1] = cat([pltpu.roll(q[16 * h:16 * h + 16], 32 * (h % 4), axis=1) if h % 4
                                    else q[16 * h:16 * h + 16] for h in range(16)])
            elif part == 1:
                k = pad_heads(r, 0.0)
                for g in range(4):
                    kn_vs[b][g, pl.ds(mul(jj, 64), 64), :] = pltpu.bitcast(
                        k[128 * g:128 * g + 128].astype(bf16).T, u32)
            else:
                vt_vs[b][jj] = pltpu.bitcast(pad_heads(r, 1.0).astype(bf16), u32)

        def proj(sb, part):
            r = proj_dot(sb, D * part, D * part + D)
            proj_post(sb, part, r)
            return ticks(r)

        scores = {}
        fresh, anchors, carry, pending = [], [], [], []

        def qk(n):
            sb, g = groups[n]
            b, jj, qs = sb[:3]
            q = [q_vs[qs][z2, 64 * g + 16 * hp:64 * g + 16 * hp + 16, :] for hp in range(4)]
            ss = []
            for c in range(4):
                k0 = max(0, rho0_of(sb) - c)
                kk = kn_vs[b][g, pl.ds(mul(jj, 64, 16 * c - 128 + 16 * k0, 16), 16 * (9 - k0)), :]
                wt = cat([lax.select(in_blk[(c + hp) % 4], q[hp], zero16) for hp in range(4)])
                ss.append((dot(pltpu.bitcast(kk, bf16), pltpu.bitcast(wt, bf16)), k0))
            scores[n] = ss
            return ticks(ss[3][0])

        def sm(n, trig):
            rho0 = rho0_of(groups[n][0])
            ss, mxs = [], []
            for s, k0 in scores.pop(n):
                m = s.shape[0]
                head = [lax.select(upper, s[0:32], neg32), s[32:m - 32]] if k0 == 0 else [s[0:m - 32]] * (m > 32)
                s = cat(head + [lax.select(upper, neg32, s[m - 32:m])])
                ss.append((s, k0))
                mxs.append(jnp.broadcast_to(jnp.max(s, axis=0, keepdims=True), (8, 128)))
            items = [(rho, c) for rho in range(rho0, 12) for c in range(4) if 0 <= rho - c <= 8]
            tix = {it: (len(trig) * i) // len(items) for i, it in enumerate(items)}
            for rho in range(rho0, 12):
                cs = [c for c in range(4) if 0 <= rho - c <= 8]
                sv, mv = [], []
                for c in cs:
                    t = anchors.pop() if anchors and rho >= ANCHOR_RHO else trig[tix[rho, c]]
                    mv += [after(t, mxs[c])] * 4
                    kk = rho - c - ss[c][1]
                    sv.append(ss[c][0][32 * kk:32 * kk + 32])
                p = pltpu.bitcast(jnp.exp2(cat(sv) - cat(mv)).astype(bf16), u32)
                p = cat([zero16] * cs[0] + [p] + [zero16] * (3 - cs[-1]))
                p = lax.select(bit0, cat([p[16:64], p[0:16]]), p)
                p = lax.select(bit1, cat([p[32:64], p[0:32]]), p)
                p_vs[n % 4][:, 16 * rho:16 * rho + 16, :] = p.reshape(4, 16, 128)

        def pv(n, defer=True):
            sb, g = groups[n] if n >= 0 else (prev, 3)
            b, jj, _, os_ = sb[:4]
            acc = [None] * 4
            tr = []
            for i in range(rho0_of(sb) // 4, 3):
                v = pltpu.bitcast(vt_vs[b][jj + i - 2, 64 * g:64 * g + 64, :], bf16)
                for hp in range(4):
                    pt = pltpu.bitcast(p_vs[n % 4][(-hp) % 4, 64 * i:64 * i + 64, :], bf16)
                    d = dot(v[32 * hp:32 * hp + 32], pt)
                    acc[hp] = d if acc[hp] is None else acc[hp] + d
                tr += ticks(d)

            def post(trig=None):
                out = []
                for hp in range(4):
                    den = acc[hp][28:29] if hp % 2 == 0 else acc[hp][0:1]
                    o = pltpu.bitcast((acc[hp] * pl.reciprocal(den, approx=False)).astype(bf16), u32)
                    if hp and trig:
                        o = cat([after(trig[2 * hp - 2 + i], o[8 * i:8 * i + 8]) for i in range(2)])
                    out.append(pltpu.roll(o, 128 - 32 * hp, axis=1) if hp else o)
                ot_vs[os_][64 * g:64 * g + 64, :] = cat(out)
            if defer:
                pending.append(post)
            else:
                post()
            return tr

        def pin():
            out_v[pl.ds(pl.multiple_of(S + 16 * z1, 16), 16), 0:128] = jnp.zeros((16, 128), bf16)
            fresh.append(pltpu.bitcast(out_v[pl.ds(pl.multiple_of(S + 16 * z2, 16), 16), 0:128], u32))

        def oproj_post(sb, y, final=False):
            b, jj, _, _, rs = sb
            rows = pl.ds(mul(jj, 128), 128)
            if b == 0:
                out_v[rows, 0:384] = y[0:384].astype(bf16).T
                rem_v[rs] = y[384:448]
                if final:
                    o_start(rows, 0, 384)
            else:
                yt = cat([rem_v[rs], y]).astype(bf16).T
                if final:
                    nr = 128 // FSPLIT
                    for i in range(FSPLIT):
                        rows = pl.ds(128 * jj + nr * i, nr)
                        out_v[rows, 384:896] = yt[nr * i:nr * i + nr]
                        o_start(rows, 384, 896)
                    return
                out_v[rows, 384:896] = yt
                o_start(rows, 0, 896)
            pin()

        def oproj(sb):
            y = dot(pltpu.bitcast(wot_v[sb[0]], bf16), pltpu.bitcast(ot_vs[sb[3]][...], bf16))
            oproj_post(sb, y)
            return ticks(y)

        def wtrans(b, part):
            lo, hi = WCOLS[part]
            wt_v[b, lo // 2:hi // 2, :] = pltpu.bitcast(w_v[b, :, lo:hi].T, u32)

        def wotrans(b):
            wot_v[b] = pltpu.bitcast(pad_heads(wo_v[b].astype(f32), 0.0).astype(bf16).T, u32)

        def flush(trig=()):
            trig = list(trig)[::2]
            for post in pending:
                post(trig[:6] if len(trig) >= 6 else None)
                trig = trig[6:]
            pending.clear()

        def slot(qks, fills, pvs, sms, drop=None, pv_first=False, hold=0):
            anchors.extend(fresh)
            fresh.clear()
            trig = list(carry)
            carry.clear()
            nc = len(trig)
            for n in qks:
                trig += qk(n)
            if not hold:
                flush(trig[nc:])
            if pv_first:
                for n in pvs:
                    trig += pv(n, False)
            nc = len(trig)
            for f in fills:
                trig += f()
            if hold == 2:
                flush(trig[nc + 8:])
            trig = trig[:len(trig) - (drop if drop is not None else (DROP if fills else 0))]
            if not pv_first:
                for n in pvs:
                    carry.extend(pv(n))
            for i, n in enumerate(sms):
                sm(n, trig[len(trig) * i // len(sms):len(trig) * (i + 1) // len(sms)])

        P = functools.partial
        if kind == "first":
            a0, a1, a2, a3 = (0, 0, 2, 2, 0), (0, 1, 1, 3, 2), (0, 2, 2, 0, 1), (0, 3, 0, 0, 1)
            b0, b1, b2 = (1, 0, 1, 2, 0), (1, 1, 2, 3, 2), (1, 2, 1, 1, 1)
            prev = None
            groups = [(sb, g) for sb in (a0, a1, a2, b0, b1, b2) for g in range(4)]
            wait(w_cp(0, 3))
            wtrans(0, 3)
            wait(x_cp(0, 0))
            r0 = proj_dot(a0, 384, 640)
            wait(x_cp(0, 1), w_cp(0, 4))
            wtrans(0, 4)
            r1 = proj_dot(a1, 384, 640)
            proj_post(a0, 1, cat([r0[64:], proj_dot(a0, 640, 896)]))
            r = cat([r1[64:], proj_dot(a1, 640, 896)])
            wait(w_cp(0, 0), x_cp(0, 2))
            wtrans(0, 0)
            proj_post(a1, 1, r)
            proj(a2, 1)
            proj_post(a0, 0, cat([proj_dot(a0, 0, 384), r0[:64]]))
            r = cat([proj_dot(a1, 0, 384), r1[:64]])
            wait(w_cp(0, 2), x_cp(0, 3))
            wtrans(0, 2)
            proj_post(a1, 0, r)
            qk(0)
            qk(1)
            held = []

            def q_a3():
                held.append(proj_dot(a3, 0, D))
                return ticks(held[0])
            slot([2, 3], [P(proj, a0, 2)], [], [0, 1])
            slot([4], [P(proj, a1, 2)], [0, 1], [2, 3])
            slot([5], [P(proj, a2, 0)], [2, 3], [4])
            slot([6], [P(proj, a2, 2)], [4], [5])
            slot([7], [P(proj, a3, 1)], [5], [6])
            slot([8], [q_a3], [6], [7], drop=DROP_BAR, pv_first=True)
            wait(x_cp(1, 0), w_cp(1, 1), w_cp(1, 0), w_cp(1, 2), wo_cp(0), wo_cp(1))
            proj_post(a3, 0, held[0])
            wtrans(1, 1)
            wtrans(1, 0)
            wtrans(1, 2)
            wotrans(0)
            wotrans(1)
            slot([9], [P(proj, b0, 1)], [7], [8], pv_first=True)
            slot([10], [P(proj, b0, 0)], [8], [9])
            slot([11], [P(proj, b1, 1)], [9], [10])
            slot([12, 13], [P(proj, b1, 0)], [10], [11])
            slot([14, 15], [P(proj, b0, 2), P(oproj, a0)], [11], [12, 13])
            slot([16], [P(proj, b1, 2)], [12, 13], [14, 15])
            slot([17], [P(proj, b2, 1)], [14, 15], [16])
            slot([18], [P(proj, b2, 0)], [], [17])
            slot([19], [P(oproj, a1)], [16, 17], [18])
            slot([20], [P(proj, b2, 2)], [18], [19])
            slot([21], [P(oproj, b0)], [19], [20])
            slot([22], [P(oproj, a2)], [20], [21])
            slot([23], [P(oproj, b1)], [21], [22], drop=DROP_PEN, hold=1)
            slot([], [P(proj, a3, 2)], [22], [23], drop=DROP_LAST, pv_first=True, hold=2)
            return

        nt = MT if kind == "mid" else LT
        seq = []
        for t in range(nt):
            seq += [(0, j + t, 0, 0, 1), (1, j + t, 1, 1, 1)]
        prev = (1, j - 1, 1, 1, 1)
        chain = [prev] + seq + [(0, j + nt, 0, 0, 1)]
        groups = [(sb, g) for sb in seq for g in range(4)]
        if kind == "last":
            groups[-4:] = groups[-4:][::-1]
        pv(-1)
        flush(qk(0))
        for i in range(len(seq)):
            lastsb = i + 1 == len(seq)
            n = 4 * i
            if not (lastsb and kind == "last"):
                slot([n + 1], [P(proj, chain[i + 2], 1)], [n - 1] if n else [], [n])
                slot([n + 2], [P(proj, chain[i + 2], 0)], [n], [n + 1])
                slot([n + 3], [P(oproj, chain[i])], [n + 1], [n + 2], drop=DROP_PEN if lastsb else None, hold=1)
                slot([] if lastsb else [n + 4], [P(proj, chain[i + 2], 2)], [n + 2], [n + 3],
                     pv_first=lastsb, drop=DROP_LAST if lastsb else None, hold=2 if lastsb else 1)
                continue
            slot([n + 1], [], [n - 1], [n])
            slot([n + 2], [], [n], [n + 1])
            slot([n + 3], [], [n + 1], [n + 2])
            flush()
            sa, sb = chain[i], seq[i]
            ot = pltpu.bitcast(ot_vs[sa[3]][...], bf16)
            y0 = dot(pltpu.bitcast(wot_v[0, 0:112], bf16), ot)
            t = pv(n + 2, False)
            y1 = dot(pltpu.bitcast(wot_v[0, 112:224], bf16), ot)
            trig = carry + ticks(y0) + t + ticks(y1)
            sm(n + 3, trig[:len(trig) - DROP_END])
            oproj_post(sa, cat([y0, y1]), True)
            pv(n + 3, False)

            def part(klo, khi, lhs_rows, top=None):
                o = ot_vs[sb[3]][klo // 2:khi // 2, :]
                if top is not None:
                    o = cat([after(top, o[0:8]), o[8:]])
                w = wot_v[1, :, klo:khi]
                return [dot(pltpu.bitcast(cat([w[r0:r1] for r0, r1 in rr]), bf16), pltpu.bitcast(o, bf16))
                        for rr in lhs_rows]
            y = cat(part(256, 512, [[(0, 112)], [(112, 224)]]))
            y = y + cat(part(128, 256, [[(0, 56)], [(56, 112)], [(112, 168)], [(168, 224)]]))
            d = part(0, 128, [[(32, 88)], [(96, 152)], [(160, 216)], [(0, 32), (88, 96), (152, 160), (216, 224)]],
                     fresh.pop())
            y = y + cat([d[3][0:64], d[0], d[3][64:80], d[1], d[3][80:96], d[2], d[3][96:112]])
            oproj_post(sb, y, True)

    @pl.when(step == 0)
    def _():
        for cps in (w_cp(0, 3), x_cp(0, 0), x_cp(0, 1), w_cp(0, 4), w_cp(0, 0), x_cp(0, 2), w_cp(0, 2),
                    x_cp(0, 3), x_cp(1, 0), w_cp(1, 1), w_cp(1, 0), w_cp(1, 2), wo_cp(0), wo_cp(1),
                    x_cp(1, 1), x_cp(0, 4), x_cp(1, 2), x_cp(0, 5)):
            for cp in cps:
                cp.start()
        body("first", 0)

    @pl.when(step == 1)
    def _():
        wait(x_cp(1, 1), x_cp(0, 4))

    @pl.when(step == 2)
    def _():
        wait(x_cp(1, 2), x_cp(0, 5))

    @pl.when(jnp.logical_and(step > 0, step <= NMID))
    def _():
        body("mid", FT + MT * (step - 1))

    @pl.when(step == NMID + 1)
    def _():
        body("last", NTILE - LT)
        wait([pltpu.make_async_copy(out_v.at[0:S], o_hbm, osem.at[0])])


@jax.jit
def pallas_concat_heads__sliding_block__sliding_block__prompt_kernel(A_x, A_wqkv, A_wo, B_x, B_wqkv, B_wo):
    xa = A_x.reshape(S, D).T
    xb = B_x.reshape(S, D).T
    anyspec = pl.BlockSpec(memory_space=pl.ANY)
    V = pltpu.VMEM
    out = pl.pallas_call(
        _kernel,
        grid=(NMID + 2,),
        in_specs=[anyspec] * 6,
        out_specs=anyspec,
        out_shape=jax.ShapeDtypeStruct((S, 2 * D), bf16),
        scratch_shapes=[
            V((2, D, 3 * D), bf16),
            V((2, D, D), bf16),
            V((2, NTILE, D, 128), bf16),
            V((2, 3 * D // 2, D), u32),
            V((2, D // 2, 512), u32),
            *[V((4, S // 2, 128), u32)] * 2,
            *[V((NTILE, 256, 128), u32)] * 2,
            *[V((1, 256, 128), u32)] * 3,
            *[V((4, 192, 128), u32)] * 4,
            *[V((256, 128), u32)] * 4,
            V((3, 64, 128), f32),
            V((S + 16, 2 * D), bf16),
            pltpu.SemaphoreType.DMA((18,)),
            pltpu.SemaphoreType.DMA((1,)),
        ],
        compiler_params=pltpu.CompilerParams(dimension_semantics=("arbitrary",),
                                             vmem_limit_bytes=64 * 1024 * 1024,
                                             disable_semaphore_checks=True,
                                             disable_bounds_checks=True),
    )(xa, A_wqkv, A_wo, xb, B_wqkv, B_wo)
    return out.reshape(1, S, 2 * D)
```

```python
import functools

import jax
import jax.numpy as jnp
from jax import lax
import jax.experimental.pallas as pl
import jax.experimental.pallas.tpu as pltpu

S, D, DH = 2048, 448, 28
NTILE = S // 128
FT = 3
MT = 4
LT = 1
NMID = (NTILE - FT - LT) // MT
assert FT + NMID * MT + LT == NTILE
NEG = -1e30
QSCALE = (DH ** -0.5) * 1.4426950408889634
f32, bf16, u32 = jnp.float32, jnp.bfloat16, jnp.uint32

DROP = 24
DROP_PEN = 20
DROP_LAST = 8
DROP_BAR = 12
DROP_END = 28
ANCHOR_RHO = 8
FSPLIT = 4

WCOLS = ((0, 384), (384, 896), (896, 1344), (384, 640), (640, 896))
XTILES = (((0, 1), (1, 2), (2, 3), (3, 4), (4, NTILE)), ((0, FT), (FT, NTILE)))


def _kernel(xa_hbm, wa_hbm, woa_hbm, xb_hbm, wb_hbm, wob_hbm, o_hbm,
            w_v, wo_v, x_v, wt_v, wot_v, kn0_v, kn1_v, vt0_v, vt1_v, q0_v, q1_v, q2_v,
            p0_v, p1_v, p2_v, p3_v, ot0_v, ot1_v, ot2_v, ot3_v, rem_v, out_v, isem, osem):
    step = pl.program_id(0)
    z1 = lax.shift_right_logical(step, 8)
    z2 = lax.shift_right_logical(step, 9)
    kn_vs, vt_vs = (kn0_v, kn1_v), (vt0_v, vt1_v)
    q_vs, p_vs, ot_vs = (q0_v, q1_v, q2_v), (p0_v, p1_v, p2_v, p3_v), (ot0_v, ot1_v, ot2_v, ot3_v)
    x_hbm, w_hbm, wo_hbm = (xa_hbm, xb_hbm), (wa_hbm, wb_hbm), (woa_hbm, wob_hbm)

    def mul(jj, m, off=0, al=None):
        v = m * jj + off
        return v if isinstance(jj, int) else pl.multiple_of(v, al or m)

    def w_cp(b, part):
        lo, hi = WCOLS[part]
        sem = {3: 1, 4: 15}.get(part, 3 * b + part)
        return [pltpu.make_async_copy(w_hbm[b].at[:, lo:hi], w_v.at[b, :, lo:hi], isem.at[sem])]

    def wo_cp(b):
        return [pltpu.make_async_copy(wo_hbm[b], wo_v.at[b], isem.at[6 + b])]

    def x_cp(b, i):
        return [pltpu.make_async_copy(x_hbm[b].at[:, 128 * t:128 * t + 128], x_v.at[b, t], isem.at[8 + 5 * b + i])
                for t in range(*XTILES[b][i])]

    def o_start(rows, lo, hi):
        pltpu.make_async_copy(out_v.at[rows, lo:hi], o_hbm.at[rows, lo:hi], osem.at[0]).start()

    def wait(*groups_of_copies):
        for cps in groups_of_copies:
            for cp in cps:
                cp.wait()

    def cat(xs):
        return xs[0] if len(xs) == 1 else jnp.concatenate(xs, axis=0)

    def dot(a, b):
        return jnp.dot(a, b, preferred_element_type=f32)

    def body(kind, j):
        blk64 = lax.broadcasted_iota(jnp.int32, (64, 128), 1) // 32
        in_blk = [lax.broadcasted_iota(jnp.int32, (16, 128), 1) // 32 == c for c in range(4)]
        bit0 = (blk64 % 2) == 1
        bit1 = blk64 >= 2
        upper = (lax.broadcasted_iota(jnp.int32, (32, 128), 0)
                 > lax.broadcasted_iota(jnp.int32, (32, 128), 1) % 32)
        never = lax.broadcasted_iota(jnp.int32, (8, 128), 0) < z1
        zero16 = jnp.zeros((16, 128), u32)
        neg32 = jnp.full((32, 128), NEG, f32)

        def ticks(x):
            return [(x, i) for i in range(x.shape[0] // 8)]

        def after(t, x):
            if isinstance(t, tuple):
                t = t[0][8 * t[1]:8 * t[1] + 8]
            if t.dtype != x.dtype:
                t = lax.bitcast_convert_type(t, x.dtype)
            return lax.select(never, t, x)

        def pad_heads(r, fill):
            lo8 = lax.broadcasted_iota(jnp.int32, (8, r.shape[1]), 0) < 4
            full = jnp.full((8, r.shape[1]), fill, f32)
            out = []
            for p in range(8):
                o = 56 * p
                sh = r[o + 24:o + 32]
                out += [r[o - 24 if p else 0:o + 24], lax.select(lo8, sh, full), lax.select(lo8, full, sh)]
            return cat(out + [r[D - 24:D]])

        def rho0_of(sb):
            jj = sb[1]
            return {0: 8, 1: 4}[jj] if isinstance(jj, int) and jj < 2 else 0

        def proj_dot(sb, lo, hi):
            b, jj = sb[:2]
            return dot(pltpu.bitcast(wt_v[b, lo // 2:hi // 2, :], bf16), x_v[b, jj])

        def proj_post(sb, part, r):
            b, jj, qs = sb[:3]
            if part == 0:
                q = pltpu.bitcast(pad_heads(r * QSCALE, 0.0).astype(bf16), u32)
                q_vs[qs][z1] = cat([pltpu.roll(q[16 * h:16 * h + 16], 32 * (h % 4), axis=1) if h % 4
                                    else q[16 * h:16 * h + 16] for h in range(16)])
            elif part == 1:
                k = pad_heads(r, 0.0)
                for g in range(4):
                    kn_vs[b][g, pl.ds(mul(jj, 64), 64), :] = pltpu.bitcast(
                        k[128 * g:128 * g + 128].astype(bf16).T, u32)
            else:
                vt_vs[b][jj] = pltpu.bitcast(pad_heads(r, 1.0).astype(bf16), u32)

        def proj(sb, part):
            r = proj_dot(sb, D * part, D * part + D)
            proj_post(sb, part, r)
            return ticks(r)

        scores = {}
        fresh, anchors, carry, pending = [], [], [], []

        def qk(n):
            sb, g = groups[n]
            b, jj, qs = sb[:3]
            q = [q_vs[qs][z2, 64 * g + 16 * hp:64 * g + 16 * hp + 16, :] for hp in range(4)]
            ss = []
            for c in range(4):
                k0 = max(0, rho0_of(sb) - c)
                kk = kn_vs[b][g, pl.ds(mul(jj, 64, 16 * c - 128 + 16 * k0, 16), 16 * (9 - k0)), :]
                wt = cat([lax.select(in_blk[(c + hp) % 4], q[hp], zero16) for hp in range(4)])
                ss.append((dot(pltpu.bitcast(kk, bf16), pltpu.bitcast(wt, bf16)), k0))
            scores[n] = ss
            return ticks(ss[3][0])

        def sm(n, trig):
            rho0 = rho0_of(groups[n][0])
            ss, mxs = [], []
            for s, k0 in scores.pop(n):
                m = s.shape[0]
                head = [lax.select(upper, s[0:32], neg32), s[32:m - 32]] if k0 == 0 else [s[0:m - 32]] * (m > 32)
                s = cat(head + [lax.select(upper, neg32, s[m - 32:m])])
                ss.append((s, k0))
                mxs.append(jnp.broadcast_to(jnp.max(s, axis=0, keepdims=True), (8, 128)))
            items = [(rho, c) for rho in range(rho0, 12) for c in range(4) if 0 <= rho - c <= 8]
            tix = {it: (len(trig) * i) // len(items) for i, it in enumerate(items)}
            for rho in range(rho0, 12):
                cs = [c for c in range(4) if 0 <= rho - c <= 8]
                sv, mv = [], []
                for c in cs:
                    t = anchors.pop() if anchors and rho >= ANCHOR_RHO else trig[tix[rho, c]]
                    mv += [after(t, mxs[c])] * 4
                    kk = rho - c - ss[c][1]
                    sv.append(ss[c][0][32 * kk:32 * kk + 32])
                p = pltpu.bitcast(jnp.exp2(cat(sv) - cat(mv)).astype(bf16), u32)
                p = cat([zero16] * cs[0] + [p] + [zero16] * (3 - cs[-1]))
                p = lax.select(bit0, cat([p[16:64], p[0:16]]), p)
                p = lax.select(bit1, cat([p[32:64], p[0:32]]), p)
                p_vs[n % 4][:, 16 * rho:16 * rho + 16, :] = p.reshape(4, 16, 128)

        def pv(n, defer=True):
            sb, g = groups[n] if n >= 0 else (prev, 3)
            b, jj, _, os_ = sb[:4]
            acc = [None] * 4
            tr = []
            for i in range(rho0_of(sb) // 4, 3):
                v = pltpu.bitcast(vt_vs[b][jj + i - 2, 64 * g:64 * g + 64, :], bf16)
                for hp in range(4):
                    pt = pltpu.bitcast(p_vs[n % 4][(-hp) % 4, 64 * i:64 * i + 64, :], bf16)
                    d = dot(v[32 * hp:32 * hp + 32], pt)
                    acc[hp] = d if acc[hp] is None else acc[hp] + d
                tr += ticks(d)

            def post(trig=None):
                out = []
                for hp in range(4):
                    den = acc[hp][28:29] if hp % 2 == 0 else acc[hp][0:1]
                    o = pltpu.bitcast((acc[hp] * pl.reciprocal(den, approx=False)).astype(bf16), u32)
                    if hp and trig:
                        o = cat([after(trig[2 * hp - 2 + i], o[8 * i:8 * i + 8]) for i in range(2)])
                    out.append(pltpu.roll(o, 128 - 32 * hp, axis=1) if hp else o)
                ot_vs[os_][64 * g:64 * g + 64, :] = cat(out)
            if defer:
                pending.append(post)
            else:
                post()
            return tr

        def pin():
            out_v[pl.ds(pl.multiple_of(S + 16 * z1, 16), 16), 0:128] = jnp.zeros((16, 128), bf16)
            fresh.append(pltpu.bitcast(out_v[pl.ds(pl.multiple_of(S + 16 * z2, 16), 16), 0:128], u32))

        def oproj_post(sb, y, final=False):
            b, jj, _, _, rs = sb
            rows = pl.ds(mul(jj, 128), 128)
            if b == 0:
                out_v[rows, 0:384] = y[0:384].astype(bf16).T
                rem_v[rs] = y[384:448]
                if final:
                    o_start(rows, 0, 384)
            else:
                yt = cat([rem_v[rs], y]).astype(bf16).T
                if final:
                    nr = 128 // FSPLIT
                    for i in range(FSPLIT):
                        rows = pl.ds(128 * jj + nr * i, nr)
                        out_v[rows, 384:896] = yt[nr * i:nr * i + nr]
                        o_start(rows, 384, 896)
                    return
                out_v[rows, 384:896] = yt
                o_start(rows, 0, 896)
            pin()

        def oproj(sb):
            y = dot(pltpu.bitcast(wot_v[sb[0]], bf16), pltpu.bitcast(ot_vs[sb[3]][...], bf16))
            oproj_post(sb, y)
            return ticks(y)

        def wtrans(b, part):
            lo, hi = WCOLS[part]
            wt_v[b, lo // 2:hi // 2, :] = pltpu.bitcast(w_v[b, :, lo:hi].T, u32)

        def wotrans(b):
            wot_v[b] = pltpu.bitcast(pad_heads(wo_v[b].astype(f32), 0.0).astype(bf16).T, u32)

        def flush(trig=()):
            trig = list(trig)[::2]
            for post in pending:
                post(trig[:6] if len(trig) >= 6 else None)
                trig = trig[6:]
            pending.clear()

        def slot(qks, fills, pvs, sms, drop=None, pv_first=False, hold=0):
            anchors.extend(fresh)
            fresh.clear()
            trig = list(carry)
            carry.clear()
            nc = len(trig)
            for n in qks:
                trig += qk(n)
            if not hold:
                flush(trig[nc:])
            if pv_first:
                for n in pvs:
                    trig += pv(n, False)
            nc = len(trig)
            for f in fills:
                trig += f()
            if hold == 2:
                flush(trig[nc + 8:])
            trig = trig[:len(trig) - (drop if drop is not None else (DROP if fills else 0))]
            if not pv_first:
                for n in pvs:
                    carry.extend(pv(n))
            for i, n in enumerate(sms):
                sm(n, trig[len(trig) * i // len(sms):len(trig) * (i + 1) // len(sms)])

        P = functools.partial
        if kind == "first":
            a0, a1, a2, a3 = (0, 0, 2, 2, 0), (0, 1, 1, 3, 2), (0, 2, 2, 0, 1), (0, 3, 0, 0, 1)
            b0, b1, b2 = (1, 0, 1, 2, 0), (1, 1, 2, 3, 2), (1, 2, 1, 1, 1)
            prev = None
            groups = [(sb, g) for sb in (a0, a1, a2, b0, b1, b2) for g in range(4)]
            wait(w_cp(0, 3))
            wtrans(0, 3)
            wait(x_cp(0, 0))
            r0 = proj_dot(a0, 384, 640)
            wait(x_cp(0, 1), w_cp(0, 4))
            wtrans(0, 4)
            r1 = proj_dot(a1, 384, 640)
            proj_post(a0, 1, cat([r0[64:], proj_dot(a0, 640, 896)]))
            r = cat([r1[64:], proj_dot(a1, 640, 896)])
            wait(w_cp(0, 0), x_cp(0, 2))
            wtrans(0, 0)
            proj_post(a1, 1, r)
            proj(a2, 1)
            proj_post(a0, 0, cat([proj_dot(a0, 0, 384), r0[:64]]))
            r = cat([proj_dot(a1, 0, 384), r1[:64]])
            wait(w_cp(0, 2), x_cp(0, 3))
            wtrans(0, 2)
            proj_post(a1, 0, r)
            qk(0)
            qk(1)
            held = []

            def q_a3():
                held.append(proj_dot(a3, 0, D))
                return ticks(held[0])
            slot([2, 3], [P(proj, a0, 2)], [], [0, 1])
            slot([4], [P(proj, a1, 2)], [0, 1], [2, 3])
            slot([5], [P(proj, a2, 0)], [2, 3], [4])
            slot([6], [P(proj, a2, 2)], [4], [5])
            slot([7], [P(proj, a3, 1)], [5], [6])
            slot([8], [q_a3], [6], [7], drop=DROP_BAR, pv_first=True)
            wait(x_cp(1, 0), w_cp(1, 1), w_cp(1, 0), w_cp(1, 2), wo_cp(0), wo_cp(1))
            proj_post(a3, 0, held[0])
            wtrans(1, 1)
            wtrans(1, 0)
            wtrans(1, 2)
            wotrans(0)
            wotrans(1)
            slot([9], [P(proj, b0, 1)], [7], [8], pv_first=True)
            slot([10], [P(proj, b0, 0)], [8], [9])
            slot([11], [P(proj, b1, 1)], [9], [10])
            slot([12, 13], [P(proj, b1, 0)], [10], [11])
            slot([14, 15], [P(proj, b0, 2), P(oproj, a0)], [11], [12, 13])
            slot([16], [P(proj, b1, 2)], [12, 13], [14, 15])
            slot([17], [P(proj, b2, 1)], [14, 15], [16])
            slot([18], [P(proj, b2, 0)], [], [17])
            slot([19], [P(oproj, a1)], [16, 17], [18])
            slot([20], [P(proj, b2, 2)], [18], [19])
            slot([21], [P(oproj, b0)], [19], [20])
            slot([22], [P(oproj, a2)], [20], [21])
            slot([23], [P(oproj, b1)], [21], [22], drop=DROP_PEN, hold=1)
            slot([], [P(proj, a3, 2)], [22], [23], drop=DROP_LAST, pv_first=True, hold=2)
            return

        nt = MT if kind == "mid" else LT
        seq = []
        for t in range(nt):
            seq += [(0, j + t, 0, 0, 1), (1, j + t, 1, 1, 1)]
        prev = (1, j - 1, 1, 1, 1)
        chain = [prev] + seq + [(0, j + nt, 0, 0, 1)]
        groups = [(sb, g) for sb in seq for g in range(4)]
        if kind == "last":
            groups[-4:] = groups[-4:][::-1]
        pv(-1)
        flush(qk(0))
        for i in range(len(seq)):
            lastsb = i + 1 == len(seq)
            n = 4 * i
            if not (lastsb and kind == "last"):
                slot([n + 1], [P(proj, chain[i + 2], 1)], [n - 1] if n else [], [n])
                slot([n + 2], [P(proj, chain[i + 2], 0)], [n], [n + 1])
                slot([n + 3], [P(oproj, chain[i])], [n + 1], [n + 2], drop=DROP_PEN if lastsb else None, hold=1)
                slot([] if lastsb else [n + 4], [P(proj, chain[i + 2], 2)], [n + 2], [n + 3],
                     pv_first=lastsb, drop=DROP_LAST if lastsb else None, hold=2 if lastsb else 1)
                continue
            slot([n + 1], [], [n - 1], [n])
            slot([n + 2], [], [n], [n + 1])
            slot([n + 3], [], [n + 1], [n + 2])
            flush()
            sa, sb = chain[i], seq[i]
            ot = pltpu.bitcast(ot_vs[sa[3]][...], bf16)
            y0 = dot(pltpu.bitcast(wot_v[0, 0:112], bf16), ot)
            t = pv(n + 2, False)
            y1 = dot(pltpu.bitcast(wot_v[0, 112:224], bf16), ot)
            trig = carry + ticks(y0) + t + ticks(y1)
            sm(n + 3, trig[:len(trig) - DROP_END])
            oproj_post(sa, cat([y0, y1]), True)
            pv(n + 3, False)

            def part(klo, khi, lhs_rows, top=None):
                o = ot_vs[sb[3]][klo // 2:khi // 2, :]
                if top is not None:
                    o = cat([after(top, o[0:8]), o[8:]])
                w = wot_v[1, :, klo:khi]
                return [dot(pltpu.bitcast(cat([w[r0:r1] for r0, r1 in rr]), bf16), pltpu.bitcast(o, bf16))
                        for rr in lhs_rows]
            y = cat(part(256, 512, [[(0, 112)], [(112, 224)]]))
            y = y + cat(part(128, 256, [[(0, 56)], [(56, 112)], [(112, 168)], [(168, 224)]]))
            d = part(0, 128, [[(32, 88)], [(96, 152)], [(160, 216)], [(0, 32), (88, 96), (152, 160), (216, 224)]],
                     fresh.pop())
            y = y + cat([d[3][0:64], d[0], d[3][64:80], d[1], d[3][80:96], d[2], d[3][96:112]])
            oproj_post(sb, y, True)

    @pl.when(step == 0)
    def _():
        for cps in (w_cp(0, 3), x_cp(0, 0), x_cp(0, 1), w_cp(0, 4), w_cp(0, 0), x_cp(0, 2), w_cp(0, 2),
                    x_cp(0, 3), x_cp(1, 0), w_cp(1, 1), w_cp(1, 0), w_cp(1, 2), wo_cp(0), wo_cp(1),
                    x_cp(1, 1), x_cp(0, 4)):
            for cp in cps:
                cp.start()
        body("first", 0)
        wait(x_cp(1, 1), x_cp(0, 4))

    body("mid", FT + MT * step)

    @pl.when(step == NMID - 1)
    def _():
        body("last", NTILE - LT)
        wait([pltpu.make_async_copy(out_v.at[0:S], o_hbm, osem.at[0])])


@jax.jit
def pallas_concat_heads__sliding_block__sliding_block__prompt_kernel(A_x, A_wqkv, A_wo, B_x, B_wqkv, B_wo):
    xa = A_x.reshape(S, D).T
    xb = B_x.reshape(S, D).T
    anyspec = pl.BlockSpec(memory_space=pl.ANY)
    V = pltpu.VMEM
    out = pl.pallas_call(
        _kernel,
        grid=(NMID,),
        in_specs=[anyspec] * 6,
        out_specs=anyspec,
        out_shape=jax.ShapeDtypeStruct((S, 2 * D), bf16),
        scratch_shapes=[
            V((2, D, 3 * D), bf16),
            V((2, D, D), bf16),
            V((2, NTILE, D, 128), bf16),
            V((2, 3 * D // 2, D), u32),
            V((2, D // 2, 512), u32),
            *[V((4, S // 2, 128), u32)] * 2,
            *[V((NTILE, 256, 128), u32)] * 2,
            *[V((1, 256, 128), u32)] * 3,
            *[V((4, 192, 128), u32)] * 4,
            *[V((256, 128), u32)] * 4,
            V((3, 64, 128), f32),
            V((S + 16, 2 * D), bf16),
            pltpu.SemaphoreType.DMA((16,)),
            pltpu.SemaphoreType.DMA((1,)),
        ],
        compiler_params=pltpu.CompilerParams(dimension_semantics=("arbitrary",),
                                             vmem_limit_bytes=64 * 1024 * 1024,
                                             disable_semaphore_checks=True,
                                             disable_bounds_checks=True),
    )(xa, A_wqkv, A_wo, xb, B_wqkv, B_wo)
    return out.reshape(1, S, 2 * D)
```

```python
import functools

import jax
import jax.numpy as jnp
from jax import lax
import jax.experimental.pallas as pl
import jax.experimental.pallas.tpu as pltpu

S, D, DH = 2048, 448, 28
NTILE = S // 128
FT = 3
MT = 4
LT = 1
NMID = (NTILE - FT - LT) // MT
assert FT + NMID * MT + LT == NTILE
NEG = -1e30
QSCALE = (DH ** -0.5) * 1.4426950408889634
f32, bf16, u32 = jnp.float32, jnp.bfloat16, jnp.uint32

DROP = 24
DROP_PEN = 20
DROP_LAST = 8
DROP_BAR = 12
DROP_END = 28
ANCHOR_RHO = 8
FSPLIT = 4

WCOLS = ((0, 384), (384, 896), (896, 1344), (384, 640), (640, 896))
XTILES = (((0, 1), (1, 2), (2, 3), (3, 4), (4, NTILE)), ((0, FT), (FT, NTILE)))


def _kernel(xa_hbm, wa_hbm, woa_hbm, xb_hbm, wb_hbm, wob_hbm, o_hbm,
            w_v, wo_v, x_v, wt_v, wot_v, kn0_v, kn1_v, vt0_v, vt1_v, q0_v, q1_v, q2_v,
            p0_v, p1_v, p2_v, p3_v, ot0_v, ot1_v, ot2_v, ot3_v, rem_v, out_v, isem, osem):
    step = pl.program_id(0)
    z1 = lax.shift_right_logical(step, 8)
    z2 = lax.shift_right_logical(step, 9)
    kn_vs, vt_vs = (kn0_v, kn1_v), (vt0_v, vt1_v)
    q_vs, p_vs, ot_vs = (q0_v, q1_v, q2_v), (p0_v, p1_v, p2_v, p3_v), (ot0_v, ot1_v, ot2_v, ot3_v)
    x_hbm, w_hbm, wo_hbm = (xa_hbm, xb_hbm), (wa_hbm, wb_hbm), (woa_hbm, wob_hbm)

    def mul(jj, m, off=0, al=None):
        v = m * jj + off
        return v if isinstance(jj, int) else pl.multiple_of(v, al or m)

    def w_cp(b, part):
        lo, hi = WCOLS[part]
        sem = {3: 1, 4: 15}.get(part, 3 * b + part)
        return [pltpu.make_async_copy(w_hbm[b].at[:, lo:hi], w_v.at[b, :, lo:hi], isem.at[sem])]

    def wo_cp(b):
        return [pltpu.make_async_copy(wo_hbm[b], wo_v.at[b], isem.at[6 + b])]

    def x_cp(b, i):
        return [pltpu.make_async_copy(x_hbm[b].at[:, 128 * t:128 * t + 128], x_v.at[b, t], isem.at[8 + 5 * b + i])
                for t in range(*XTILES[b][i])]

    def o_start(rows, lo, hi):
        pltpu.make_async_copy(out_v.at[rows, lo:hi], o_hbm.at[rows, lo:hi], osem.at[0]).start()

    def wait(*groups_of_copies):
        for cps in groups_of_copies:
            for cp in cps:
                cp.wait()

    def cat(xs):
        return xs[0] if len(xs) == 1 else jnp.concatenate(xs, axis=0)

    def dot(a, b):
        return jnp.dot(a, b, preferred_element_type=f32)

    def body(kind, j):
        blk64 = lax.broadcasted_iota(jnp.int32, (64, 128), 1) // 32
        in_blk = [lax.broadcasted_iota(jnp.int32, (16, 128), 1) // 32 == c for c in range(4)]
        bit0 = (blk64 % 2) == 1
        bit1 = blk64 >= 2
        upper = (lax.broadcasted_iota(jnp.int32, (32, 128), 0)
                 > lax.broadcasted_iota(jnp.int32, (32, 128), 1) % 32)
        never = lax.broadcasted_iota(jnp.int32, (8, 128), 0) < z1
        zero16 = jnp.zeros((16, 128), u32)
        neg32 = jnp.full((32, 128), NEG, f32)

        def ticks(x):
            return [(x, i) for i in range(x.shape[0] // 8)]

        def after(t, x):
            if isinstance(t, tuple):
                t = t[0][8 * t[1]:8 * t[1] + 8]
            if t.dtype != x.dtype:
                t = lax.bitcast_convert_type(t, x.dtype)
            return lax.select(never, t, x)

        def pad_heads(r, fill):
            lo8 = lax.broadcasted_iota(jnp.int32, (8, r.shape[1]), 0) < 4
            full = jnp.full((8, r.shape[1]), fill, f32)
            out = []
            for p in range(8):
                o = 56 * p
                sh = r[o + 24:o + 32]
                out += [r[o - 24 if p else 0:o + 24], lax.select(lo8, sh, full), lax.select(lo8, full, sh)]
            return cat(out + [r[D - 24:D]])

        def rho0_of(sb):
            jj = sb[1]
            return {0: 8, 1: 4}[jj] if isinstance(jj, int) and jj < 2 else 0

        def proj_dot(sb, lo, hi):
            b, jj = sb[:2]
            return dot(pltpu.bitcast(wt_v[b, lo // 2:hi // 2, :], bf16), x_v[b, jj])

        def proj_post(sb, part, r):
            b, jj, qs = sb[:3]
            if part == 0:
                q = pltpu.bitcast(pad_heads(r * QSCALE, 0.0).astype(bf16), u32)
                q_vs[qs][z1] = cat([pltpu.roll(q[16 * h:16 * h + 16], 32 * (h % 4), axis=1) if h % 4
                                    else q[16 * h:16 * h + 16] for h in range(16)])
            elif part == 1:
                k = pad_heads(r, 0.0)
                for g in range(4):
                    kn_vs[b][g, pl.ds(mul(jj, 64), 64), :] = pltpu.bitcast(
                        k[128 * g:128 * g + 128].astype(bf16).T, u32)
            else:
                vt_vs[b][jj] = pltpu.bitcast(pad_heads(r, 1.0).astype(bf16), u32)

        def proj(sb, part):
            r = proj_dot(sb, D * part, D * part + D)
            proj_post(sb, part, r)
            return ticks(r)

        scores = {}
        fresh, anchors, carry, pending = [], [], [], []

        def qk(n):
            sb, g = groups[n]
            b, jj, qs = sb[:3]
            q = [q_vs[qs][z2, 64 * g + 16 * hp:64 * g + 16 * hp + 16, :] for hp in range(4)]
            ss = []
            for c in range(4):
                k0 = max(0, rho0_of(sb) - c)
                kk = kn_vs[b][g, pl.ds(mul(jj, 64, 16 * c - 128 + 16 * k0, 16), 16 * (9 - k0)), :]
                wt = cat([lax.select(in_blk[(c + hp) % 4], q[hp], zero16) for hp in range(4)])
                ss.append((dot(pltpu.bitcast(kk, bf16), pltpu.bitcast(wt, bf16)), k0))
            scores[n] = ss
            return ticks(ss[3][0])

        def sm(n, trig):
            rho0 = rho0_of(groups[n][0])
            ss, mxs = [], []
            for s, k0 in scores.pop(n):
                m = s.shape[0]
                head = [lax.select(upper, s[0:32], neg32), s[32:m - 32]] if k0 == 0 else [s[0:m - 32]] * (m > 32)
                s = cat(head + [lax.select(upper, neg32, s[m - 32:m])])
                ss.append((s, k0))
                mxs.append(jnp.broadcast_to(jnp.max(s, axis=0, keepdims=True), (8, 128)))
            items = [(rho, c) for rho in range(rho0, 12) for c in range(4) if 0 <= rho - c <= 8]
            tix = {it: (len(trig) * i) // len(items) for i, it in enumerate(items)}
            for rho in range(rho0, 12):
                cs = [c for c in range(4) if 0 <= rho - c <= 8]
                sv, mv = [], []
                for c in cs:
                    t = anchors.pop() if anchors and rho >= ANCHOR_RHO else trig[tix[rho, c]]
                    mv += [after(t, mxs[c])] * 4
                    kk = rho - c - ss[c][1]
                    sv.append(ss[c][0][32 * kk:32 * kk + 32])
                p = pltpu.bitcast(jnp.exp2(cat(sv) - cat(mv)).astype(bf16), u32)
                p = cat([zero16] * cs[0] + [p] + [zero16] * (3 - cs[-1]))
                p = lax.select(bit0, cat([p[16:64], p[0:16]]), p)
                p = lax.select(bit1, cat([p[32:64], p[0:32]]), p)
                p_vs[n % 4][:, 16 * rho:16 * rho + 16, :] = p.reshape(4, 16, 128)

        def pv(n, defer=True):
            sb, g = groups[n] if n >= 0 else (prev, 3)
            b, jj, _, os_ = sb[:4]
            acc = [None] * 4
            tr = []
            for i in range(rho0_of(sb) // 4, 3):
                v = pltpu.bitcast(vt_vs[b][jj + i - 2, 64 * g:64 * g + 64, :], bf16)
                for hp in range(4):
                    pt = pltpu.bitcast(p_vs[n % 4][(-hp) % 4, 64 * i:64 * i + 64, :], bf16)
                    d = dot(v[32 * hp:32 * hp + 32], pt)
                    acc[hp] = d if acc[hp] is None else acc[hp] + d
                tr += ticks(d)

            def post(trig=None):
                out = []
                for hp in range(4):
                    den = acc[hp][28:29] if hp % 2 == 0 else acc[hp][0:1]
                    o = pltpu.bitcast((acc[hp] * pl.reciprocal(den, approx=False)).astype(bf16), u32)
                    if hp and trig:
                        o = cat([after(trig[2 * hp - 2 + i], o[8 * i:8 * i + 8]) for i in range(2)])
                    out.append(pltpu.roll(o, 128 - 32 * hp, axis=1) if hp else o)
                ot_vs[os_][64 * g:64 * g + 64, :] = cat(out)
            if defer:
                pending.append(post)
            else:
                post()
            return tr

        def pin():
            out_v[pl.ds(pl.multiple_of(S + 16 * z1, 16), 16), 0:128] = jnp.zeros((16, 128), bf16)
            fresh.append(pltpu.bitcast(out_v[pl.ds(pl.multiple_of(S + 16 * z2, 16), 16), 0:128], u32))

        def oproj_post(sb, y, final=False):
            b, jj, _, _, rs = sb
            rows = pl.ds(mul(jj, 128), 128)
            if b == 0:
                out_v[rows, 0:384] = y[0:384].astype(bf16).T
                rem_v[rs] = y[384:448]
                if final:
                    o_start(rows, 0, 384)
            else:
                yt = cat([rem_v[rs], y]).astype(bf16).T
                if final:
                    nr = 128 // FSPLIT
                    for i in range(FSPLIT):
                        rows = pl.ds(128 * jj + nr * i, nr)
                        out_v[rows, 384:896] = yt[nr * i:nr * i + nr]
                        o_start(rows, 384, 896)
                    return
                out_v[rows, 384:896] = yt
                o_start(rows, 0, 896)
            pin()

        def oproj(sb):
            y = dot(pltpu.bitcast(wot_v[sb[0]], bf16), pltpu.bitcast(ot_vs[sb[3]][...], bf16))
            oproj_post(sb, y)
            return ticks(y)

        def wtrans(b, part):
            lo, hi = WCOLS[part]
            wt_v[b, lo // 2:hi // 2, :] = pltpu.bitcast(w_v[b, :, lo:hi].T, u32)

        def wotrans(b):
            wot_v[b] = pltpu.bitcast(pad_heads(wo_v[b].astype(f32), 0.0).astype(bf16).T, u32)

        def flush(trig=()):
            trig = list(trig)[::2]
            for post in pending:
                post(trig[:6] if len(trig) >= 6 else None)
                trig = trig[6:]
            pending.clear()

        def slot(qks, fills, pvs, sms, drop=None, pv_first=False, hold=0):
            anchors.extend(fresh)
            fresh.clear()
            trig = list(carry)
            carry.clear()
            nc = len(trig)
            for n in qks:
                trig += qk(n)
            if not hold:
                flush(trig[nc:])
            if pv_first:
                for n in pvs:
                    trig += pv(n, False)
            nc = len(trig)
            for f in fills:
                trig += f()
            if hold == 2:
                flush(trig[nc + 8:])
            trig = trig[:len(trig) - (drop if drop is not None else (DROP if fills else 0))]
            if not pv_first:
                for n in pvs:
                    carry.extend(pv(n))
            for i, n in enumerate(sms):
                sm(n, trig[len(trig) * i // len(sms):len(trig) * (i + 1) // len(sms)])

        P = functools.partial
        if kind == "first":
            a0, a1, a2, a3 = (0, 0, 2, 2, 0), (0, 1, 1, 3, 2), (0, 2, 2, 0, 1), (0, 3, 0, 0, 1)
            b0, b1, b2 = (1, 0, 1, 2, 0), (1, 1, 2, 3, 2), (1, 2, 1, 1, 1)
            prev = None
            groups = [(sb, g) for sb in (a0, a1, a2, b0, b1, b2) for g in range(4)]
            wait(w_cp(0, 3))
            wtrans(0, 3)
            wait(x_cp(0, 0), x_cp(0, 1))
            r0 = proj_dot(a0, 384, 640)
            r1 = proj_dot(a1, 384, 640)
            wait(w_cp(0, 4), x_cp(0, 2))
            wtrans(0, 4)
            r2 = proj_dot(a2, 384, 640)
            proj_post(a0, 1, cat([r0[64:], proj_dot(a0, 640, 896)]))
            r = cat([r1[64:], proj_dot(a1, 640, 896)])
            wait(w_cp(0, 0))
            wtrans(0, 0)
            proj_post(a1, 1, r)
            proj_post(a2, 1, cat([r2[64:], proj_dot(a2, 640, 896)]))
            proj_post(a0, 0, cat([proj_dot(a0, 0, 384), r0[:64]]))
            r = cat([proj_dot(a1, 0, 384), r1[:64]])

            def q_a2():
                t = proj_dot(a2, 0, 384)
                proj_post(a2, 0, cat([t, r2[:64]]))
                return ticks(t)
            wait(w_cp(0, 2), x_cp(0, 3))
            wtrans(0, 2)
            proj_post(a1, 0, r)
            qk(0)
            qk(1)
            held = []

            def q_a3():
                held.append(proj_dot(a3, 0, D))
                return ticks(held[0])
            slot([2, 3], [P(proj, a0, 2)], [], [0, 1])
            slot([4], [P(proj, a1, 2)], [0, 1], [2, 3])
            slot([5], [q_a2], [2, 3], [4])
            slot([6], [P(proj, a2, 2)], [4], [5])
            slot([7], [P(proj, a3, 1)], [5], [6])
            slot([8], [], [6], [7])
            slot([9], [q_a3], [7], [8], drop=DROP_BAR, pv_first=True)
            wait(x_cp(1, 0), w_cp(1, 1), w_cp(1, 0), w_cp(1, 2), wo_cp(0), wo_cp(1))
            proj_post(a3, 0, held[0])
            wtrans(1, 1)
            wtrans(1, 0)
            wtrans(1, 2)
            wotrans(0)
            wotrans(1)
            slot([10], [P(proj, b0, 1)], [8], [9], pv_first=True)
            slot([11], [P(proj, b0, 0)], [9], [10])
            slot([], [P(proj, b1, 1), P(proj, b1, 0), P(qk, 12), P(qk, 13)], [10], [11])
            slot([14, 15], [P(proj, b0, 2), P(oproj, a0)], [11], [12, 13])
            slot([16], [P(proj, b1, 2)], [12, 13], [14, 15])
            slot([17], [P(proj, b2, 1)], [14, 15], [16])
            slot([18], [P(proj, b2, 0)], [], [17])
            slot([19], [P(oproj, a1)], [16, 17], [18])
            slot([20], [P(proj, b2, 2)], [18], [19])
            slot([21], [P(oproj, b0)], [19], [20])
            slot([22], [P(oproj, a2)], [20], [21])
            slot([23], [P(oproj, b1)], [21], [22], drop=DROP_PEN, hold=1)
            slot([], [P(proj, a3, 2)], [22], [23], drop=DROP_LAST, pv_first=True, hold=2)
            return

        nt = MT if kind == "mid" else LT
        seq = []
        for t in range(nt):
            seq += [(0, j + t, 0, 0, 1), (1, j + t, 1, 1, 1)]
        prev = (1, j - 1, 1, 1, 1)
        chain = [prev] + seq + [(0, j + nt, 0, 0, 1)]
        groups = [(sb, g) for sb in seq for g in range(4)]
        if kind == "last":
            groups[-4:] = groups[-4:][::-1]
        pv(-1)
        flush(qk(0))
        for i in range(len(seq)):
            lastsb = i + 1 == len(seq)
            n = 4 * i
            if not (lastsb and kind == "last"):
                slot([n + 1], [P(proj, chain[i + 2], 1)], [n - 1] if n else [], [n])
                slot([n + 2], [P(proj, chain[i + 2], 0)], [n], [n + 1])
                slot([n + 3], [P(oproj, chain[i])], [n + 1], [n + 2], drop=DROP_PEN if lastsb else None, hold=1)
                slot([] if lastsb else [n + 4], [P(proj, chain[i + 2], 2)], [n + 2], [n + 3],
                     pv_first=lastsb, drop=DROP_LAST if lastsb else None, hold=2 if lastsb else 1)
                continue
            slot([n + 1], [], [n - 1], [n])
            slot([n + 2], [], [n], [n + 1])
            slot([n + 3], [], [n + 1], [n + 2])
            flush()
            sa, sb = chain[i], seq[i]
            ot = pltpu.bitcast(ot_vs[sa[3]][...], bf16)
            y0 = dot(pltpu.bitcast(wot_v[0, 0:112], bf16), ot)
            t = pv(n + 2, False)
            y1 = dot(pltpu.bitcast(wot_v[0, 112:224], bf16), ot)
            trig = carry + ticks(y0) + t + ticks(y1)
            sm(n + 3, trig[:len(trig) - DROP_END])
            oproj_post(sa, cat([y0, y1]), True)
            pv(n + 3, False)

            def part(klo, khi, lhs_rows, top=None):
                o = ot_vs[sb[3]][klo // 2:khi // 2, :]
                if top is not None:
                    o = cat([after(top, o[0:8]), o[8:]])
                w = wot_v[1, :, klo:khi]
                return [dot(pltpu.bitcast(cat([w[r0:r1] for r0, r1 in rr]), bf16), pltpu.bitcast(o, bf16))
                        for rr in lhs_rows]
            y = cat(part(256, 512, [[(0, 112)], [(112, 224)]]))
            y = y + cat(part(128, 256, [[(0, 56)], [(56, 112)], [(112, 168)], [(168, 224)]]))
            d = part(0, 128, [[(32, 88)], [(96, 152)], [(160, 216)], [(0, 32), (88, 96), (152, 160), (216, 224)]],
                     fresh.pop())
            y = y + cat([d[3][0:64], d[0], d[3][64:80], d[1], d[3][80:96], d[2], d[3][96:112]])
            oproj_post(sb, y, True)

    @pl.when(step == 0)
    def _():
        for cps in (w_cp(0, 3), x_cp(0, 0), x_cp(0, 1), w_cp(0, 4), x_cp(0, 2), w_cp(0, 0), w_cp(0, 2),
                    x_cp(0, 3), x_cp(1, 0), w_cp(1, 1), w_cp(1, 0), w_cp(1, 2), wo_cp(0), wo_cp(1),
                    x_cp(1, 1), x_cp(0, 4)):
            for cp in cps:
                cp.start()
        body("first", 0)
        wait(x_cp(1, 1), x_cp(0, 4))

    body("mid", FT + MT * step)

    @pl.when(step == NMID - 1)
    def _():
        body("last", NTILE - LT)
        wait([pltpu.make_async_copy(out_v.at[0:S], o_hbm, osem.at[0])])


@jax.jit
def pallas_concat_heads__sliding_block__sliding_block__prompt_kernel(A_x, A_wqkv, A_wo, B_x, B_wqkv, B_wo):
    xa = A_x.reshape(S, D).T
    xb = B_x.reshape(S, D).T
    anyspec = pl.BlockSpec(memory_space=pl.ANY)
    V = pltpu.VMEM
    out = pl.pallas_call(
        _kernel,
        grid=(NMID,),
        in_specs=[anyspec] * 6,
        out_specs=anyspec,
        out_shape=jax.ShapeDtypeStruct((S, 2 * D), bf16),
        scratch_shapes=[
            V((2, D, 3 * D), bf16),
            V((2, D, D), bf16),
            V((2, NTILE, D, 128), bf16),
            V((2, 3 * D // 2, D), u32),
            V((2, D // 2, 512), u32),
            *[V((4, S // 2, 128), u32)] * 2,
            *[V((NTILE, 256, 128), u32)] * 2,
            *[V((1, 256, 128), u32)] * 3,
            *[V((4, 192, 128), u32)] * 4,
            *[V((256, 128), u32)] * 4,
            V((3, 64, 128), f32),
            V((S + 16, 2 * D), bf16),
            pltpu.SemaphoreType.DMA((16,)),
            pltpu.SemaphoreType.DMA((1,)),
        ],
        compiler_params=pltpu.CompilerParams(dimension_semantics=("arbitrary",),
                                             vmem_limit_bytes=64 * 1024 * 1024,
                                             disable_semaphore_checks=True,
                                             disable_bounds_checks=True),
    )(xa, A_wqkv, A_wo, xb, B_wqkv, B_wo)
    return out.reshape(1, S, 2 * D)
```
